```python
import jax
import jax.numpy as jnp

def _softmax(x, axis=-1):
    return jax.nn.softmax(x, axis=axis)
def _gelu(x):
    return jax.nn.gelu(x, approximate=True)
def _silu(x):
    return jax.nn.silu(x)
def _sigmoid(x):
    return jax.nn.sigmoid(x)
def _layernorm(x, axis=-1, eps=1e-5):
    m = jnp.mean(x, axis=axis, keepdims=True)
    v = jnp.var(x, axis=axis, keepdims=True)
    return (x - m) / jnp.sqrt(v + eps)
def _scatter_add(tgt, idx, src, axis=0):
    return tgt.at[idx].add(src)
def _segment_sum(src, seg, n):
    return jax.ops.segment_sum(src, seg, n)
class _Rng:
    def __init__(self, key):
        self._k = key
    def _next(self):
        self._k, sub = jax.random.split(self._k)
        return sub
    def normal(self, shape):
        return jax.random.normal(self._next(), shape, dtype=jnp.bfloat16)
    def randint(self, lo, hi, shape):
        return jax.random.randint(self._next(), shape, lo, hi, dtype=jnp.int32)
    def uniform(self, shape, lo=0.0, hi=1.0):
        return jax.random.uniform(self._next(), shape, jnp.bfloat16, lo, hi)
    def permutation(self, n):
        return jax.random.permutation(self._next(), n)


kernel_name = 'concat_heads__sliding_block_cached__compressed_kv_cla__decode'

def setup_inputs():
    _rng = _Rng(jax.random.key(int.from_bytes(__import__("os").urandom(4), "little")))
    _w = (lambda a: (lambda t: t.astype(jnp.bfloat16) if jnp.issubdtype(t.dtype, jnp.floating) else t)(jnp.asarray(a)))
    def _A_setup():
        B, Sq, D = 4, 1, 512
        Hq, Hkv, Sk, Dh = 32, 32, 4096, 128
        assert Hq % Hkv == 0, (Hq, Hkv)
        return {
            "x": _w((lambda *s: _rng.normal(s) * 0.05)(B, Sq, D)),
            "k_cache": _w((lambda *s: _rng.normal(s) * 0.05)(B, Hkv, Sk, Dh)),
            "v_cache": _w((lambda *s: _rng.normal(s) * 0.05)(B, Hkv, Sk, Dh)),
            "wq": _w((lambda *s: _rng.normal(s) * 0.05)(D, Hq * Dh) * (D ** -0.5)),
            "wo": _w((lambda *s: _rng.normal(s) * 0.05)(Hq * Dh, D) * ((Hq * Dh) ** -0.5)),
        }
    _A_in = _A_setup()

    def _B_setup():
        B, H, Sq, Sk, D, M = 4, 32, 1, 4096, 128, 512
        Dc = 4 * D
        return {
            "x": _w((lambda *s: _rng.normal(s) * 0.05)(B, Sq, M)),
            "c_kv": _w((lambda *s: _rng.normal(s) * 0.05)(B, Sk, Dc)),
            "w_q": _w((lambda *s: _rng.normal(s) * 0.05)(M, H, D) * (M ** -0.5)),
            "w_uk": _w((lambda *s: _rng.normal(s) * 0.05)(Dc, H, D) * (Dc ** -0.5)),
            "w_uv": _w((lambda *s: _rng.normal(s) * 0.05)(Dc, H, D) * (Dc ** -0.5)),
            "w_o": _w((lambda *s: _rng.normal(s) * 0.05)(H, D, M) * ((H * D) ** -0.5)),
        }
    _B_in = _B_setup()

    return {
        "A_x": _A_in["x"],
        "A_k_cache": _A_in["k_cache"],
        "A_v_cache": _A_in["v_cache"],
        "A_wq": _A_in["wq"],
        "A_wo": _A_in["wo"],
        "B_x": _B_in["x"],
        "B_c_kv": _B_in["c_kv"],
        "B_w_q": _B_in["w_q"],
        "B_w_uk": _B_in["w_uk"],
        "B_w_uv": _B_in["w_uv"],
        "B_w_o": _B_in["w_o"],
    }

def reference(A_x, A_k_cache, A_v_cache, A_wq, A_wo, B_x, B_c_kv, B_w_q, B_w_uk, B_w_uv, B_w_o):
    def _A_ref(x, k_cache, v_cache, wq, wo):
        B, Sq, D = x.shape
        Hq, Dh = 32, 128
        Hkv, Sk = k_cache.shape[1], k_cache.shape[2]
        W = min(4096, max(256, Sk // 4))
        rep = Hq // Hkv
        q = (lambda x, *d: x.transpose(*d))((x @ wq).reshape(B, Sq, Hq, Dh), 0, 2, 1, 3)
        k = jnp.repeat(k_cache[:, :, Sk - W:, :], rep, axis=1)
        v = jnp.repeat(v_cache[:, :, Sk - W:, :], rep, axis=1)
        scores = jnp.einsum("bhqd,bhkd->bhqk", q, k) * (Dh ** -0.5)
        p = _softmax(scores, axis=-1)
        o = jnp.einsum("bhqk,bhkd->bhqd", p, v)
        return (lambda x, *d: x.transpose(*d))(o, 0, 2, 1, 3).reshape(B, Sq, Hq * Dh) @ wo

    def _B_ref(x, c_kv, w_q, w_uk, w_uv, w_o):
        B, Sq, M = x.shape[0], x.shape[1], x.shape[2]
        Sk = c_kv.shape[1]
        H, D = w_q.shape[1], w_q.shape[2]
        q = jnp.einsum("bqm,mhd->bhqd", x, w_q)
        k = jnp.einsum("bkc,chd->bhkd", c_kv, w_uk)
        v = jnp.einsum("bkc,chd->bhkd", c_kv, w_uv)
        scores = jnp.einsum("bhqd,bhkd->bhqk", q, k) * (D ** -0.5)
        off = Sk - Sq
        qi = jnp.arange(Sq)[:, None]
        kj = jnp.arange(Sk)[None, :]
        cmask = kj <= (qi + off)
        scores = jnp.where(cmask[None, None], scores, -1e9)
        p = _softmax(scores, axis=-1)
        ctx = jnp.einsum("bhqk,bhkd->bhqd", p, v)
        return jnp.einsum("bhqd,hdm->bqm", ctx, w_o)

    a = _A_ref(A_x, A_k_cache, A_v_cache, A_wq, A_wo)
    b = _B_ref(B_x, B_c_kv, B_w_q, B_w_uk, B_w_uv, B_w_o)
    return jnp.concatenate([a, b], axis=-1)
```

```python
import functools

import jax
import jax.numpy as jnp
from jax import lax
from jax.experimental import pallas as pl
from jax.experimental.pallas import tpu as pltpu

BF = jnp.bfloat16
F32 = jnp.float32
U32 = jnp.uint32

NB = 4
NH = 32
DH = 128
SK = 4096
WIN = 1024
DM = 512
SCALE = float(DH) ** -0.5

DEPTH = 8
NSEM = 16
KV_SLOTS = 8
HI_NUM, HI_DEN = 3, 8

_NT = (((1,), (1,)), ((), ()))


def _split_pair(w):
    lo = pltpu.bitcast(w << 16, F32).astype(BF)
    hi = pltpu.bitcast(w & U32(0xFFFF0000), F32).astype(BF)
    return lo, hi


def _kernel(ax_hbm, k_hbm, v_hbm, awq_hbm, awo_hbm,
            bx_hbm, c_hbm, bwq_hbm, bwuk_hbm, bwuv_hbm, bwo_hbm,
            out_ref,
            x_v, kbuf, vbuf, awq_v, awo_v, c_v, bwq_v, bwuk_v, bwuv_v, bwo_v,
            x8_s, qb_s, qabs_s, qabs_b, s_s, acc_s, cx_s, ctx_s, qa_s, qa_b, o_s, outb_s,
            sems, xsems, *, compute):

    def rows_unit(hbm, vmem, rows):
        hi = rows * HI_NUM // HI_DEN

        def parts(i):
            r0 = i * rows if isinstance(i, int) else pl.multiple_of(i * rows, rows)
            return [(hbm.at[pl.ds(r0, hi), :], vmem.at[pl.ds(r0, hi), :]),
                    (hbm.at[pl.ds(r0 + hi, rows - hi), :], vmem.at[pl.ds(r0 + hi, rows - hi), :]),
                    vmem.at[pl.ds(r0, rows), :]]
        return parts

    def awq_parts(i):
        hi = 128 * HI_NUM // HI_DEN
        if isinstance(i, int):
            r0, c0 = (i % 4) * 128, (i // 4) * 1024
        else:
            r0 = pl.multiple_of((i % 4) * 128, 128)
            c0 = pl.multiple_of((i // 4) * 1024, 1024)
        return [(awq_hbm.at[pl.ds(r0, hi), pl.ds(c0, 1024)], awq_v.at[i, pl.ds(0, hi), :]),
                (awq_hbm.at[pl.ds(r0 + hi, 128 - hi), pl.ds(c0, 1024)], awq_v.at[i, pl.ds(hi, 128 - hi), :]),
                awq_v.at[i]]

    def kv_parts(g, is_v):
        hbm, buf = (v_hbm, vbuf) if is_v else (k_hbm, kbuf)
        hi = WIN * HI_NUM // HI_DEN
        slot = g % KV_SLOTS
        return [(hbm.at[g, pl.ds(SK - WIN, hi), :], buf.at[slot, pl.ds(0, hi), :]),
                (hbm.at[g, pl.ds(SK - WIN + hi, WIN - hi), :], buf.at[slot, pl.ds(hi, WIN - hi), :]),
                buf.at[slot]]

    def start_parts(parts, sem):
        pltpu.make_async_copy(parts[0][0], parts[0][1], sem).start(priority=0)
        pltpu.make_async_copy(parts[1][0], parts[1][1], sem).start(priority=1)

    def wait_parts(parts, sem):
        pltpu.make_async_copy(parts[2], parts[2], sem).wait()

    phases = [
        ("bwq", 16, lambda i, p: rows_unit(bwq_hbm, bwq_v, 1024)(i)),
        ("bwuk", 16, lambda i, p: rows_unit(bwuk_hbm, bwuk_v, 1024)(i)),
        ("c", 64, lambda i, p: rows_unit(c_hbm, c_v, 256)(i)),
        ("awq", 16, lambda i, p: awq_parts(i)),
        ("bwuv", 16, lambda i, p: rows_unit(bwuv_hbm, bwuv_v, 1024)(i)),
        ("bwo", 16, lambda i, p: rows_unit(bwo_hbm, bwo_v, 256)(i)),
        ("kv", 256, lambda i, p: kv_parts(i // 2, p == 1)),
        ("awo", 16, lambda i, p: rows_unit(awo_hbm, awo_v, 256)(i)),
    ]
    pidx = {p[0]: n for n, p in enumerate(phases)}

    def start_unit(ph, i, parity):
        start_parts(phases[ph][2](i, parity), sems.at[i % NSEM])

    def step(name, i, parity):
        ph = pidx[name]
        n = phases[ph][1]
        wait_parts(phases[ph][2](i, parity), sems.at[i % NSEM])
        j = i + DEPTH
        last = ph + 1 == len(phases)
        if isinstance(i, int):
            if j < n:
                start_unit(ph, j, parity)
            elif not last:
                start_unit(ph + 1, j - n, parity)
        else:
            pl.when(j < n)(lambda: start_unit(ph, j, parity))
            if not last:
                pl.when(j >= n)(lambda: start_unit(ph + 1, j - n, parity))

    for i in range(DEPTH):
        start_unit(0, i, i % 2)
    cxa = pltpu.make_async_copy(ax_hbm, x_v.at[0], xsems.at[0])
    cxb = pltpu.make_async_copy(bx_hbm, x_v.at[1], xsems.at[1])
    cxa.start()
    cxb.start()
    qb_s[...] = jnp.zeros_like(qb_s)
    ctx_s[...] = jnp.zeros_like(ctx_s)
    cx_s[...] = jnp.zeros_like(cx_s)
    o_s[...] = jnp.zeros_like(o_s)
    qa_s[...] = jnp.zeros_like(qa_s)
    cxa.wait()
    cxb.wait()
    row8 = lax.broadcasted_iota(jnp.int32, (8, DM), 0)
    for t in range(2):
        x8 = jnp.zeros((8, DM), F32)
        for b in range(NB):
            xb = jnp.broadcast_to(x_v[t, b].astype(F32), (8, DM))
            x8 = jnp.where(row8 == b, xb, x8)
        for j in range(4):
            x8_s[t, j] = x8[:, j * 128:(j + 1) * 128].astype(BF)

    def head_pair(w_v, j, hp):
        w32 = w_v.bitcast(U32)
        wj = w32.at[pl.ds(pl.multiple_of(j * 2048, 2048), 2048), :]
        return _split_pair(wj[pl.ds(hp, 128, stride=16), :])

    def grouped(name, body):
        def it(j, carry):
            for s in range(4):
                step(name, j * 4 + s, s % 2)
            if compute:
                body(j)
            return carry
        lax.fori_loop(0, 4, it, 0)

    def bwq_body(j):
        x = x8_s[1, j]
        for hp in range(16):
            lo, hi = head_pair(bwq_v, j, hp)
            qb_s[2 * hp] += jnp.dot(x, lo, preferred_element_type=F32)
            qb_s[2 * hp + 1] += jnp.dot(x, hi, preferred_element_type=F32)
    grouped("bwq", bwq_body)

    def bwuk_body(j):
        for hp in range(16):
            lo, hi = head_pair(bwuk_v, j, hp)
            for h, w in ((2 * hp, lo), (2 * hp + 1, hi)):
                qabs_s[j, pl.ds(8 * h, 8), :] = lax.dot_general(
                    qb_s[h].astype(BF), w, _NT, preferred_element_type=F32)
    grouped("bwuk", bwuk_body)

    if compute:
        for b in range(NB):
            for j in range(4):
                qabs_b[b, :, j * 128:(j + 1) * 128] = qabs_s[j, pl.ds(b, NH, stride=8), :].astype(BF)

    def c_chunk(u):
        return c_v[pl.ds(pl.multiple_of(u * 256, 256), 256), :]

    def b_scores(b, j, m):
        s = lax.dot_general(qabs_b[b], c_chunk(b * 16 + j), _NT, preferred_element_type=F32)
        s_s[b % 2, j] = s
        return jnp.maximum(m, jnp.maximum(s[:, :128], s[:, 128:]))

    def b_values(b, j, mx, l):
        p = jnp.exp((s_s[b % 2, j] - mx) * SCALE)
        acc_s[...] += jnp.dot(p.astype(BF), c_chunk(b * 16 + j), preferred_element_type=F32)
        return l + p[:, :128] + p[:, 128:]

    def b_finish(b, l):
        inv = 1.0 / jnp.sum(l, axis=-1, keepdims=True)
        ctxc = acc_s[...] * inv
        for j in range(4):
            cx_s[j, pl.ds(b * NH, NH), :] = ctxc[:, j * 128:(j + 1) * 128]

    neg = jnp.full((NH, 128), -jnp.inf, F32)
    zero = jnp.zeros((NH, 128), F32)
    m_prev = None
    for b in range(NB + 1):
        if b > 0 and compute:
            mx = jnp.max(m_prev, axis=-1, keepdims=True)
            acc_s[...] = jnp.zeros_like(acc_s)

        def it(jj, carry, b=b):
            m, l = carry
            for s in range(2):
                j = jj * 2 + s
                if b < NB:
                    step("c", b * 16 + j, s)
                else:
                    step("awq", j, s)
                if compute:
                    if b < NB:
                        m = b_scores(b, j, m)
                    else:
                        cb = j // 4
                        qa_s[cb] += jnp.dot(x8_s[0, j % 4], awq_v[j], preferred_element_type=F32)
                    if b > 0:
                        l = b_values(b - 1, j, mx, l)
            return m, l
        m_prev, l_fin = lax.fori_loop(0, 8, it, (neg, zero))
        if b > 0 and compute:
            b_finish(b - 1, l_fin)

    if compute:
        for h in range(NH):
            qa_b[h] = qa_s[h // 8, :, (h % 8) * 128:(h % 8 + 1) * 128].astype(BF)

    def bwuv_body(j):
        for hp in range(16):
            lo, hi = head_pair(bwuv_v, j, hp)
            for h, w in ((2 * hp, lo), (2 * hp + 1, hi)):
                lhs = cx_s[j, pl.ds(h, 8, stride=NH), :].astype(BF)
                ctx_s[h] += jnp.dot(lhs, w, preferred_element_type=F32)
    grouped("bwuv", bwuv_body)

    def out_proj(name, w_v, src):
        def it(jj, acc):
            for s in range(2):
                u = jj * 2 + s
                step(name, u, s)
                if compute:
                    lhs = jnp.concatenate([src[2 * u], src[2 * u + 1]], axis=1).astype(BF)
                    w = w_v[pl.ds(pl.multiple_of(u * 256, 256), 256), :]
                    acc = acc + jnp.dot(lhs, w, preferred_element_type=F32)
            return acc
        return lax.fori_loop(0, 8, it, jnp.zeros((8, DM), F32))

    outb_s[...] = out_proj("bwo", bwo_v, ctx_s)

    row = lax.broadcasted_iota(jnp.int32, (8, DH), 0)

    def kv_it(g, carry):
        b = g // NH
        h = g % NH
        slot = g % KV_SLOTS
        step("kv", 2 * g, 0)
        if compute:
            s = lax.dot_general(qa_b[h], kbuf[slot], _NT, preferred_element_type=F32)
            m = jnp.max(s, axis=-1, keepdims=True)
            p = jnp.exp((s - m) * SCALE)
            inv = 1.0 / jnp.sum(p, axis=-1, keepdims=True)
            p = p.astype(BF)
        step("kv", 2 * g + 1, 1)
        if compute:
            o = jnp.dot(p, vbuf[slot], preferred_element_type=F32) * inv
            o_s[h] = jnp.where(row == b, o, o_s[h])
        return carry
    lax.fori_loop(0, NB * NH, kv_it, 0)

    outa = out_proj("awo", awo_v, o_s)
    res = jnp.concatenate([outa, outb_s[...]], axis=1)
    for b in range(NB):
        out_ref[b] = res[b:b + 1, :].astype(out_ref.dtype)


def _build(compute=True):
    vm = pltpu.VMEM
    scratch = [
        vm((2, NB, 1, DM), BF),
        vm((KV_SLOTS, WIN, DH), BF),
        vm((KV_SLOTS, WIN, DH), BF),
        vm((16, 128, 1024), BF),
        vm((NH * DH, DM), BF),
        vm((NB * SK, DM), BF),
        vm((DM * NH, DH), BF),
        vm((DM * NH, DH), BF),
        vm((DM * NH, DH), BF),
        vm((NH * DH, DM), BF),
        vm((2, 4, 8, 128), BF),
        vm((NH, 8, DH), F32),
        vm((4, NH * 8, 128), F32),
        vm((NB, NH, DM), BF),
        vm((2, 16, NH, 256), F32),
        vm((NH, DM), F32),
        vm((4, 8 * NH, 128), F32),
        vm((NH, 8, DH), F32),
        vm((4, 8, 1024), F32),
        vm((NH, 8, DH), BF),
        vm((NH, 8, DH), F32),
        vm((8, DM), F32),
        pltpu.SemaphoreType.DMA((NSEM,)),
        pltpu.SemaphoreType.DMA((2,)),
    ]
    return pl.pallas_call(
        functools.partial(_kernel, compute=compute),
        out_shape=jax.ShapeDtypeStruct((NB, 1, 2 * DM), BF),
        in_specs=[pl.BlockSpec(memory_space=pl.ANY)] * 11,
        out_specs=pl.BlockSpec(memory_space=pltpu.VMEM),
        scratch_shapes=scratch,
        compiler_params=pltpu.CompilerParams(vmem_limit_bytes=64 * 1024 * 1024),
    )


def _run(compute, A_x, A_k_cache, A_v_cache, A_wq, A_wo, B_x, B_c_kv, B_w_q, B_w_uk, B_w_uv, B_w_o):
    return _build(compute)(
        A_x,
        A_k_cache.reshape(NB * NH, SK, DH),
        A_v_cache.reshape(NB * NH, SK, DH),
        A_wq, A_wo,
        B_x,
        B_c_kv.reshape(NB * SK, DM),
        B_w_q.reshape(DM * NH, DH),
        B_w_uk.reshape(DM * NH, DH),
        B_w_uv.reshape(DM * NH, DH),
        B_w_o.reshape(NH * DH, DM),
    )


@jax.jit
def pallas_concat_heads__sliding_block_cached__compressed_kv_cla__decode_kernel(
    A_x: jax.Array,
    A_k_cache: jax.Array,
    A_v_cache: jax.Array,
    A_wq: jax.Array,
    A_wo: jax.Array,
    B_x: jax.Array,
    B_c_kv: jax.Array,
    B_w_q: jax.Array,
    B_w_uk: jax.Array,
    B_w_uv: jax.Array,
    B_w_o: jax.Array,
):
    return _run(True, A_x, A_k_cache, A_v_cache, A_wq, A_wo, B_x, B_c_kv, B_w_q, B_w_uk, B_w_uv, B_w_o)
```

```python
import functools

import jax
import jax.numpy as jnp
from jax import lax
from jax.experimental import pallas as pl
from jax.experimental.pallas import tpu as pltpu

BF = jnp.bfloat16
F32 = jnp.float32
U32 = jnp.uint32

NB = 4
NH = 32
DH = 128
SK = 4096
WIN = 1024
DM = 512
SCALE = float(DH) ** -0.5

DEPTH = 8
NSEM = 16
KV_SLOTS = 8
HI_NUM, HI_DEN = 3, 8

_NT = (((1,), (1,)), ((), ()))


def _split_pair(w):
    lo = pltpu.bitcast(w << 16, F32).astype(BF)
    hi = pltpu.bitcast(w & U32(0xFFFF0000), F32).astype(BF)
    return lo, hi


def _kernel(ax_hbm, k_hbm, v_hbm, awq_hbm, awo_hbm,
            bx_hbm, c_hbm, bwq_hbm, bwuk_hbm, bwuv_hbm, bwo_hbm,
            out_ref,
            x_v, kbuf, vbuf, awq_v, awo_v, c_v, bwq_v, bwuk_v, bwuv_v, bwo_v,
            x8_s, qb_s, qabs_s, qabs_b, s_s, acc_s, cx_s, ctx_s, qa_s, qa_b, o_s, outb_s,
            sems, xsems, *, compute):

    def rows_unit(hbm, vmem, rows):
        hi = rows * HI_NUM // HI_DEN

        def parts(i):
            r0 = i * rows if isinstance(i, int) else pl.multiple_of(i * rows, rows)
            return [(hbm.at[pl.ds(r0, hi), :], vmem.at[pl.ds(r0, hi), :]),
                    (hbm.at[pl.ds(r0 + hi, rows - hi), :], vmem.at[pl.ds(r0 + hi, rows - hi), :]),
                    vmem.at[pl.ds(r0, rows), :]]
        return parts

    def awq_parts(i):
        hi = 128 * HI_NUM // HI_DEN
        if isinstance(i, int):
            r0, c0 = (i % 4) * 128, (i // 4) * 1024
        else:
            r0 = pl.multiple_of((i % 4) * 128, 128)
            c0 = pl.multiple_of((i // 4) * 1024, 1024)
        return [(awq_hbm.at[pl.ds(r0, hi), pl.ds(c0, 1024)], awq_v.at[i, pl.ds(0, hi), :]),
                (awq_hbm.at[pl.ds(r0 + hi, 128 - hi), pl.ds(c0, 1024)], awq_v.at[i, pl.ds(hi, 128 - hi), :]),
                awq_v.at[i]]

    def kv_parts(g, is_v):
        hbm, buf = (v_hbm, vbuf) if is_v else (k_hbm, kbuf)
        hi = WIN * HI_NUM // HI_DEN
        slot = g % KV_SLOTS
        return [(hbm.at[g, pl.ds(SK - WIN, hi), :], buf.at[slot, pl.ds(0, hi), :]),
                (hbm.at[g, pl.ds(SK - WIN + hi, WIN - hi), :], buf.at[slot, pl.ds(hi, WIN - hi), :]),
                buf.at[slot]]

    def start_parts(parts, sem):
        pltpu.make_async_copy(parts[0][0], parts[0][1], sem).start(priority=0)
        pltpu.make_async_copy(parts[1][0], parts[1][1], sem).start(priority=1)

    def wait_parts(parts, sem):
        pltpu.make_async_copy(parts[2], parts[2], sem).wait()

    phases = [
        ("bwq", 16, lambda i, p: rows_unit(bwq_hbm, bwq_v, 1024)(i)),
        ("bwuk", 16, lambda i, p: rows_unit(bwuk_hbm, bwuk_v, 1024)(i)),
        ("c", 64, lambda i, p: rows_unit(c_hbm, c_v, 256)(i)),
        ("awq", 16, lambda i, p: awq_parts(i)),
        ("bwuv", 16, lambda i, p: rows_unit(bwuv_hbm, bwuv_v, 1024)(i)),
        ("bwo", 16, lambda i, p: rows_unit(bwo_hbm, bwo_v, 256)(i)),
        ("kv", 256, lambda i, p: kv_parts(i // 2, p == 1)),
        ("awo", 16, lambda i, p: rows_unit(awo_hbm, awo_v, 256)(i)),
    ]
    pidx = {p[0]: n for n, p in enumerate(phases)}

    def start_unit(ph, i, parity):
        start_parts(phases[ph][2](i, parity), sems.at[i % NSEM])

    def step(name, i, parity):
        ph = pidx[name]
        n = phases[ph][1]
        wait_parts(phases[ph][2](i, parity), sems.at[i % NSEM])
        j = i + DEPTH
        last = ph + 1 == len(phases)
        if isinstance(i, int):
            if j < n:
                start_unit(ph, j, parity)
            elif not last:
                start_unit(ph + 1, j - n, parity)
        else:
            pl.when(j < n)(lambda: start_unit(ph, j, parity))
            if not last:
                pl.when(j >= n)(lambda: start_unit(ph + 1, j - n, parity))

    for i in range(DEPTH):
        start_unit(0, i, i % 2)
    cxa = pltpu.make_async_copy(ax_hbm, x_v.at[0], xsems.at[0])
    cxb = pltpu.make_async_copy(bx_hbm, x_v.at[1], xsems.at[1])
    cxa.start()
    cxb.start()
    qb_s[...] = jnp.zeros_like(qb_s)
    ctx_s[...] = jnp.zeros_like(ctx_s)
    cx_s[...] = jnp.zeros_like(cx_s)
    o_s[...] = jnp.zeros_like(o_s)
    qa_s[...] = jnp.zeros_like(qa_s)
    cxa.wait()
    cxb.wait()
    for t in range(2):
        x8 = jnp.concatenate([x_v[t].astype(F32), jnp.zeros((8 - NB, DM), F32)], axis=0)
        for j in range(4):
            x8_s[t, j] = x8[:, j * 128:(j + 1) * 128].astype(BF)

    def head_pair(w_v, j, hp):
        w32 = w_v.bitcast(U32)
        wj = w32.at[pl.ds(pl.multiple_of(j * 2048, 2048), 2048), :]
        return _split_pair(wj[pl.ds(hp, 128, stride=16), :])

    def grouped(name, body):
        def it(j, carry):
            for s in range(4):
                step(name, j * 4 + s, s % 2)
            if compute:
                body(j)
            return carry
        lax.fori_loop(0, 4, it, 0)

    def bwq_body(j):
        x = x8_s[1, j]
        for hp in range(16):
            lo, hi = head_pair(bwq_v, j, hp)
            qb_s[2 * hp] += jnp.dot(x, lo, preferred_element_type=F32)
            qb_s[2 * hp + 1] += jnp.dot(x, hi, preferred_element_type=F32)
    grouped("bwq", bwq_body)

    def bwuk_body(j):
        for hp in range(16):
            lo, hi = head_pair(bwuk_v, j, hp)
            for h, w in ((2 * hp, lo), (2 * hp + 1, hi)):
                qabs_s[j, pl.ds(8 * h, 8), :] = lax.dot_general(
                    qb_s[h].astype(BF), w, _NT, preferred_element_type=F32)
    grouped("bwuk", bwuk_body)

    if compute:
        for b in range(NB):
            for j in range(4):
                qabs_b[b, :, j * 128:(j + 1) * 128] = qabs_s[j, pl.ds(b, NH, stride=8), :].astype(BF)

    def c_chunk(u):
        return c_v[pl.ds(pl.multiple_of(u * 256, 256), 256), :]

    def b_scores(b, j, m):
        s = lax.dot_general(qabs_b[b], c_chunk(b * 16 + j), _NT, preferred_element_type=F32)
        s_s[b % 2, j] = s
        return jnp.maximum(m, jnp.maximum(s[:, :128], s[:, 128:]))

    def b_values(b, j, mx, l):
        p = jnp.exp((s_s[b % 2, j] - mx) * SCALE)
        acc_s[...] += jnp.dot(p.astype(BF), c_chunk(b * 16 + j), preferred_element_type=F32)
        return l + p[:, :128] + p[:, 128:]

    def b_finish(b, l):
        inv = 1.0 / jnp.sum(l, axis=-1, keepdims=True)
        ctxc = acc_s[...] * inv
        for j in range(4):
            cx_s[j, pl.ds(b * NH, NH), :] = ctxc[:, j * 128:(j + 1) * 128]

    neg = jnp.full((NH, 128), -jnp.inf, F32)
    zero = jnp.zeros((NH, 128), F32)
    m_prev = None
    for b in range(NB + 1):
        if b > 0 and compute:
            mx = jnp.max(m_prev, axis=-1, keepdims=True)
            acc_s[...] = jnp.zeros_like(acc_s)

        def it(jj, carry, b=b):
            m, l = carry
            for s in range(2):
                j = jj * 2 + s
                if b < NB:
                    step("c", b * 16 + j, s)
                else:
                    step("awq", j, s)
                if compute:
                    if b < NB:
                        m = b_scores(b, j, m)
                    else:
                        cb = j // 4
                        qa_s[cb] += jnp.dot(x8_s[0, j % 4], awq_v[j], preferred_element_type=F32)
                    if b > 0:
                        l = b_values(b - 1, j, mx, l)
            return m, l
        m_prev, l_fin = lax.fori_loop(0, 8, it, (neg, zero))
        if b > 0 and compute:
            b_finish(b - 1, l_fin)

    if compute:
        for h in range(NH):
            qa_b[h] = qa_s[h // 8, :, (h % 8) * 128:(h % 8 + 1) * 128].astype(BF)

    def bwuv_body(j):
        for hp in range(16):
            lo, hi = head_pair(bwuv_v, j, hp)
            for h, w in ((2 * hp, lo), (2 * hp + 1, hi)):
                lhs = cx_s[j, pl.ds(h, 8, stride=NH), :].astype(BF)
                ctx_s[h] += jnp.dot(lhs, w, preferred_element_type=F32)
    grouped("bwuv", bwuv_body)

    def out_proj(name, w_v, src):
        def it(jj, acc):
            for s in range(2):
                u = jj * 2 + s
                step(name, u, s)
                if compute:
                    lhs = jnp.concatenate([src[2 * u], src[2 * u + 1]], axis=1).astype(BF)
                    w = w_v[pl.ds(pl.multiple_of(u * 256, 256), 256), :]
                    acc = acc + jnp.dot(lhs, w, preferred_element_type=F32)
            return acc
        return lax.fori_loop(0, 8, it, jnp.zeros((8, DM), F32))

    outb_s[...] = out_proj("bwo", bwo_v, ctx_s)

    row = lax.broadcasted_iota(jnp.int32, (8, DH), 0)

    def kv_it(g, carry):
        b = g // NH
        h = g % NH
        slot = g % KV_SLOTS
        step("kv", 2 * g, 0)
        if compute:
            s = lax.dot_general(qa_b[h], kbuf[slot], _NT, preferred_element_type=F32)
            m = jnp.max(s, axis=-1, keepdims=True)
            p = jnp.exp((s - m) * SCALE)
            inv = 1.0 / jnp.sum(p, axis=-1, keepdims=True)
            p = p.astype(BF)
        step("kv", 2 * g + 1, 1)
        if compute:
            o = jnp.dot(p, vbuf[slot], preferred_element_type=F32) * inv
            o_s[h] = jnp.where(row == b, o, o_s[h])
        return carry
    lax.fori_loop(0, NB * NH, kv_it, 0)

    outa = out_proj("awo", awo_v, o_s)
    res = jnp.concatenate([outa, outb_s[...]], axis=1)
    out_ref[...] = res[:NB, :].astype(out_ref.dtype)


def _build(compute=True):
    vm = pltpu.VMEM
    scratch = [
        vm((2, NB, DM), BF),
        vm((KV_SLOTS, WIN, DH), BF),
        vm((KV_SLOTS, WIN, DH), BF),
        vm((16, 128, 1024), BF),
        vm((NH * DH, DM), BF),
        vm((NB * SK, DM), BF),
        vm((DM * NH, DH), BF),
        vm((DM * NH, DH), BF),
        vm((DM * NH, DH), BF),
        vm((NH * DH, DM), BF),
        vm((2, 4, 8, 128), BF),
        vm((NH, 8, DH), F32),
        vm((4, NH * 8, 128), F32),
        vm((NB, NH, DM), BF),
        vm((2, 16, NH, 256), F32),
        vm((NH, DM), F32),
        vm((4, 8 * NH, 128), F32),
        vm((NH, 8, DH), F32),
        vm((4, 8, 1024), F32),
        vm((NH, 8, DH), BF),
        vm((NH, 8, DH), F32),
        vm((8, DM), F32),
        pltpu.SemaphoreType.DMA((NSEM,)),
        pltpu.SemaphoreType.DMA((2,)),
    ]
    return pl.pallas_call(
        functools.partial(_kernel, compute=compute),
        out_shape=jax.ShapeDtypeStruct((NB, 2 * DM), BF),
        in_specs=[pl.BlockSpec(memory_space=pl.ANY)] * 11,
        out_specs=pl.BlockSpec(memory_space=pltpu.VMEM),
        scratch_shapes=scratch,
        compiler_params=pltpu.CompilerParams(vmem_limit_bytes=64 * 1024 * 1024),
    )


def _run(compute, A_x, A_k_cache, A_v_cache, A_wq, A_wo, B_x, B_c_kv, B_w_q, B_w_uk, B_w_uv, B_w_o):
    out = _build(compute)(
        A_x.reshape(NB, DM),
        A_k_cache.reshape(NB * NH, SK, DH),
        A_v_cache.reshape(NB * NH, SK, DH),
        A_wq, A_wo,
        B_x.reshape(NB, DM),
        B_c_kv.reshape(NB * SK, DM),
        B_w_q.reshape(DM * NH, DH),
        B_w_uk.reshape(DM * NH, DH),
        B_w_uv.reshape(DM * NH, DH),
        B_w_o.reshape(NH * DH, DM),
    )
    return out.reshape(NB, 1, 2 * DM)


@jax.jit
def pallas_concat_heads__sliding_block_cached__compressed_kv_cla__decode_kernel(
    A_x: jax.Array,
    A_k_cache: jax.Array,
    A_v_cache: jax.Array,
    A_wq: jax.Array,
    A_wo: jax.Array,
    B_x: jax.Array,
    B_c_kv: jax.Array,
    B_w_q: jax.Array,
    B_w_uk: jax.Array,
    B_w_uv: jax.Array,
    B_w_o: jax.Array,
):
    return _run(True, A_x, A_k_cache, A_v_cache, A_wq, A_wo, B_x, B_c_kv, B_w_q, B_w_uk, B_w_uv, B_w_o)
```

```python
import functools

import jax
import jax.numpy as jnp
from jax import lax
from jax.experimental import pallas as pl
from jax.experimental.pallas import tpu as pltpu

BF = jnp.bfloat16
F32 = jnp.float32
U32 = jnp.uint32

NB = 4
NH = 32
DH = 128
SK = 4096
WIN = 1024
DM = 512
SCALE = float(DH) ** -0.5

KV_SLOTS = 16
LAG = 2

CUT_A = 15
CUT_B = 17

_NT = (((1,), (1,)), ((), ()))

CFG = dict(compute=True, wide="rows", fence=True)


def _split_pair(w):
    lo = pltpu.bitcast(w << 16, F32).astype(BF)
    hi = pltpu.bitcast(w & U32(0xFFFF0000), F32).astype(BF)
    return lo, hi


def _tile_runs(t0, t1, per_row):
    runs = []
    while t0 < t1:
        r, c = divmod(t0, per_row)
        if c == 0 and t1 - t0 >= per_row:
            n = (t1 - t0) // per_row
            runs.append((r, n, 0, per_row))
            t0 += n * per_row
        else:
            n = min(per_row - c, t1 - t0)
            runs.append((r, 1, c, n))
            t0 += n
    return runs


def _unit_pieces(cut, per_row):
    if CFG["wide"] == "rows" and 1 < per_row < 32:
        cut = (cut + per_row // 2) // per_row * per_row
    lo = [_tile_runs(cut + 32 * p, cut + 32 * (p + 1), per_row) for p in range(3)]
    unit = per_row if per_row < 32 else 1
    mid = ((cut + 96 + 128) // 2 + unit - 1) // unit * unit
    hi = [_tile_runs(0, cut, per_row), _tile_runs(cut + 96, mid, per_row), _tile_runs(mid, 128, per_row)]
    return lo, hi


def _kernel(ax_hbm, k_hbm, v_hbm, awq_hbm, awo_hbm,
            bx_hbm, c_hbm, bwq_hbm, bwuk_hbm, bwuv_hbm, bwo_hbm,
            out_ref,
            x_v, kbuf, vbuf, awq_v, awo_v, c_v, bwq_v, bwuk_v, bwuv_v, bwo_v,
            x8_s, qb_s, qabs_s, qabs_b, s_s, m_s, l_s, acc_s, cx_s, ctx_s,
            qa_s, qa_b, sa_s, ma_s, p_s, la_s, o_s, out_s, one_s,
            lo_sems, hi_sems, xsems):
    compute = CFG["compute"]

    def mat_unit(it, u):
        return 2 * ((it & 3) + 4 * (u & 1)) + (it >> 2)

    def aligned(x, m):
        return x if isinstance(x, int) else pl.multiple_of(x, m)

    def lead(hbm, vmem, cut, per_row, src_row0=0):
        def rect(si, di, run):
            r, n, c, m = run
            cols = pl.ds(c * 128, m * 128)
            return (hbm.at[si, pl.ds(src_row0 + 8 * r, 8 * n), cols],
                    vmem.at[di, pl.ds(8 * r, 8 * n), cols])
        return rect, _unit_pieces(cut, per_row)

    def flat(hbm, vmem, cut, per_row):
        rows = 8 * 128 // per_row

        def rect(si, di, run):
            r, n, c, m = run
            rs = pl.ds(aligned(si * rows + 8 * r, 8), 8 * n)
            cols = pl.ds(c * 128, m * 128)
            return hbm.at[rs, cols], vmem.at[rs, cols]
        return rect, _unit_pieces(cut, per_row)

    arr = dict(
        bwq=flat(bwq_hbm, bwq_v, CUT_B, 1),
        bwuk=flat(bwuk_hbm, bwuk_v, CUT_B, 1),
        bwuv=flat(bwuv_hbm, bwuv_v, CUT_B, 1),
        awq=flat(awq_hbm, awq_v, CUT_A, 32),
        c=lead(c_hbm, c_v, CUT_B, 4),
        bwo=lead(bwo_hbm, bwo_v, CUT_B, 4),
        awo=lead(awo_hbm, awo_v, CUT_A, 4),
        k=lead(k_hbm, kbuf, CUT_A, 1, SK - WIN),
        v=lead(v_hbm, vbuf, CUT_A, 1, SK - WIN),
    )

    def pair_phase(a, b):
        def unit(it, u):
            i = mat_unit(it, u)
            return (a if u < 2 else b), i, i
        return unit

    def c_phase(it, u):
        i = 16 * u + 2 * (it & 7) + (it >> 3)
        return "c", i, i

    def kv_phase(it, u):
        g = 2 * it + (u >> 1)
        return ("v" if u & 1 else "k"), g, g & (KV_SLOTS - 1)

    phases = [(0, 8, pair_phase("bwq", "awq")),
              (8, 8, pair_phase("bwuk", "bwuv")),
              (16, 16, c_phase),
              (32, 64, kv_phase),
              (96, 8, pair_phase("bwo", "awo"))]
    NIT = 104

    def phase_of(j):
        for n, (j0, cnt, _) in enumerate(phases):
            if j0 <= j < j0 + cnt:
                return n
        return None

    def copies(ph, j, t, high):
        j0, _, unit = phases[ph]
        name, si, di = unit(j - j0, (t + 2) % 4 if high else t % 4)
        rect, pieces = arr[name]
        sem = hi_sems.at[j & 3] if high else lo_sems.at[(j & 3) * 16 + t]
        out = []
        for run in pieces[1 if high else 0][t // 4]:
            src, dst = rect(si, di, run)
            out.append(pltpu.make_async_copy(src, dst, sem))
        return out

    def start_tick(ph, j, t):
        for cp in copies(ph, j, t, True):
            cp.start(priority=0)
        for cp in copies(ph, j, t, False):
            cp.start(priority=1)

    def wait_tick(ph, j, t):
        if t == 0:
            for tt in range(12):
                for cp in copies(ph, j, tt, True):
                    cp.wait()
        for cp in copies(ph, j, t, False):
            cp.wait()

    def run_job(job, j):
        name = getattr(job, "__qualname__", "job").split(".")[-3 if job.__name__ == "job" else -1]
        if not compute or name in CFG.get("skip", ()):
            return
        if CFG.get("scopes") == "job":
            with jax.named_scope(name):
                job(j)
        elif CFG["fence"]:
            pl.when(one_s[0] > 0)(lambda: job(j))
        else:
            job(j)

    def iteration(j, sph, wphs, jobs):
        for t in range(12):
            if len(wphs) == 1:
                wait_tick(wphs[0], j - LAG, t)
            elif len(wphs) == 2:
                edge = phases[wphs[1]][0] + LAG
                pl.when(j < edge)(lambda: wait_tick(wphs[0], j - LAG, t))
                pl.when(j >= edge)(lambda: wait_tick(wphs[1], j - LAG, t))
            if sph is not None:
                start_tick(sph, j, t)
            for job in jobs.get(t, ()):
                run_job(job, j)

    def segment(j0, j1, jobs):
        sph = phase_of(j0)
        assert all(phase_of(j) == sph for j in range(j0, j1))
        wphs = sorted({phase_of(j - LAG) for j in range(j0, j1) if j >= LAG})
        if CFG.get("scopes") == "seg":
            with jax.named_scope(f"seg{j0:03d}_{j1 - j0}"):
                _segment(j0, j1, sph, wphs, jobs)
        else:
            _segment(j0, j1, sph, wphs, jobs)

    def _segment(j0, j1, sph, wphs, jobs):
        if j1 - j0 == 1:
            iteration(j0, sph, wphs, jobs)
        else:
            def body(j, carry):
                iteration(j, sph, wphs, jobs)
                return carry
            lax.fori_loop(j0, j1, body, 0)

    def head_pair(w_v, ch, hp):
        w32 = w_v.bitcast(U32)
        wj = w32.at[pl.ds(aligned(ch * 2048, 2048), 2048), :]
        return _split_pair(wj[pl.ds(hp, 128, stride=16), :])

    def wq_job(j0, q):
        def job(j):
            ch = j - j0
            x = x8_s[1, ch]
            for hp in range(4 * q, 4 * q + 4):
                lo, hi = head_pair(bwq_v, ch, hp)
                qb_s[2 * hp] += jnp.dot(x, lo, preferred_element_type=F32)
                qb_s[2 * hp + 1] += jnp.dot(x, hi, preferred_element_type=F32)
        return job

    def awq_job(j0, q):
        def job(j):
            half = j - j0
            cols = pl.ds(aligned(half * 2048, 2048), 2048)
            qa_s[half] += jnp.dot(x8_s[0, q], awq_v[pl.ds(q * 128, 128), cols],
                                  preferred_element_type=F32)
            if q == 3:
                for hh in range(16):
                    qa_b[half * 16 + hh] = qa_s[half, :, hh * 128:(hh + 1) * 128].astype(BF)
        return job

    def wuk_job(j0, q):
        def job(j):
            ch = j - j0
            for hp in range(4 * q, 4 * q + 4):
                lo, hi = head_pair(bwuk_v, ch, hp)
                for h, w in ((2 * hp, lo), (2 * hp + 1, hi)):
                    qabs_s[pl.ds(8 * h, 8), :] = lax.dot_general(
                        qb_s[h].astype(BF), w, _NT, preferred_element_type=F32)
            if q == 3:
                for b in range(NB):
                    qabs_b[b, ch] = qabs_s[pl.ds(b, NH, stride=8), :].astype(BF)
        return job

    def bqk_job(index):
        def job(j):
            n = index(j)
            b = n & 3
            k = n >> 2
            i = 16 * b + 2 * (k & 7) + (k >> 3)
            q = jnp.concatenate([qabs_b[b, ch] for ch in range(4)], axis=1)
            s = lax.dot_general(q, c_v[i], _NT, preferred_element_type=F32)
            s_s[i] = s
            m_s[b] = jnp.maximum(m_s[b], jnp.maximum(s[:, :128], s[:, 128:]))
        return job

    def bmax_job(j):
        for b in range(NB):
            m_s[b] = jnp.broadcast_to(jnp.max(m_s[b], axis=-1, keepdims=True), (NH, 128))

    def bpv_job(index):
        def job(j):
            i = index(j)
            b = i >> 4
            m = m_s[b]
            s = s_s[i]
            p0 = jnp.exp((s[:, :128] - m) * SCALE)
            p1 = jnp.exp((s[:, 128:] - m) * SCALE)
            l_s[b] += p0 + p1
            p = jnp.concatenate([p0, p1], axis=1).astype(BF)
            acc_s[b] += jnp.dot(p, c_v[i], preferred_element_type=F32)
        return job

    def bfin_job(j):
        for b in range(NB):
            ctxc = acc_s[b] * (1.0 / jnp.sum(l_s[b], axis=-1, keepdims=True))
            for ch in range(4):
                cx_s[ch, pl.ds(b * NH, NH), :] = ctxc[:, ch * 128:(ch + 1) * 128]

    def wuv_job(j0, q):
        def job(j):
            ch = j - j0
            for hp in range(4 * q, 4 * q + 4):
                lo, hi = head_pair(bwuv_v, ch, hp)
                for h, w in ((2 * hp, lo), (2 * hp + 1, hi)):
                    lhs = cx_s[ch, pl.ds(h, 8, stride=NH), :].astype(BF)
                    ctx_s[h] += jnp.dot(lhs, w, preferred_element_type=F32)
        return job

    row = lax.broadcasted_iota(jnp.int32, (8, DH), 0)

    def a_scores(g, e):
        s = lax.dot_general(qa_b[g & (NH - 1)], kbuf[g & (KV_SLOTS - 1)], _NT,
                            preferred_element_type=F32)
        sa_s[e] = s
        parts = [s[:, c * 128:(c + 1) * 128] for c in range(8)]
        while len(parts) > 1:
            parts = [jnp.maximum(parts[2 * c], parts[2 * c + 1]) for c in range(len(parts) // 2)]
        ma_s[e] = parts[0]

    def a_softmax(e):
        m = jnp.max(ma_s[e], axis=-1, keepdims=True)
        p = jnp.exp((sa_s[e] - m) * SCALE)
        p_s[e] = p.astype(BF)
        parts = [p[:, c * 128:(c + 1) * 128] for c in range(8)]
        while len(parts) > 1:
            parts = [parts[2 * c] + parts[2 * c + 1] for c in range(len(parts) // 2)]
        la_s[e] = parts[0]

    def a_values(g, e):
        o = jnp.dot(p_s[e], vbuf[g & (KV_SLOTS - 1)], preferred_element_type=F32)
        inv = 1.0 / jnp.sum(la_s[e], axis=-1, keepdims=True)
        h = g & (NH - 1)
        o_s[h] = jnp.where(row == (g >> 5), o * inv, o_s[h])

    def a_job(e, stages="qsv", also=None):
        def job(j):
            g = 2 * (j - 35) + e
            if "v" in stages:
                a_values(g - 2, e)
            if also is not None:
                also(j)
            if "q" in stages:
                a_scores(g, e)
            if "s" in stages:
                a_softmax(1 - e)
        return job

    def proj(side, i, halves=(0, 1)):
        w_v, src = ((awo_v, o_s), (bwo_v, ctx_s))[side]
        acc = None
        for hf in halves:
            d = jnp.dot(src[2 * i + hf].astype(BF), w_v[i, pl.ds(hf * 128, 128), :],
                        preferred_element_type=F32)
            acc = d if acc is None else acc + d
        return acc

    def proj_job(side, lag):
        def job(j):
            it = j - lag - 96
            out_s[side] += proj(side, mat_unit(it, 0)) + proj(side, mat_unit(it, 1))
        return job

    cxa = pltpu.make_async_copy(ax_hbm, x_v.at[0], xsems.at[0])
    cxb = pltpu.make_async_copy(bx_hbm, x_v.at[1], xsems.at[1])
    for j in range(LAG):
        for t in range(12):
            start_tick(0, j, t)
            if j == 0 and t == 1:
                cxa.start()
                cxb.start()
    one_s[0] = 1
    for r in (qb_s, qa_s, l_s, acc_s, cx_s, ctx_s, sa_s, ma_s, p_s, o_s, out_s):
        r[...] = jnp.zeros_like(r)
    la_s[...] = jnp.ones_like(la_s)
    for slot in (KV_SLOTS - 2, KV_SLOTS - 1):
        vbuf[slot] = jnp.zeros((WIN, DH), BF)
    m_s[...] = jnp.full(m_s.shape, -jnp.inf, F32)
    cxa.wait()
    cxb.wait()
    for t in range(2):
        x8 = jnp.concatenate([x_v[t].astype(F32), jnp.zeros((8 - NB, DM), F32)], axis=0)
        for ch in range(4):
            x8_s[t, ch] = x8[:, ch * 128:(ch + 1) * 128].astype(BF)

    def four(mk):
        return {3 * q + 2: [mk(q)] for q in range(4)}

    def with_a(x0=None, x1=None):
        mode = CFG.get("amode", "merged")
        if mode == "merged":
            jobs = {2: [a_job(0)], 8: [a_job(1)]}
            if x0 is not None:
                jobs[5] = [x0]
                jobs[11] = [x1]
        else:
            jobs = {2: [a_job(0, "v", x0)], 5: [a_job(0, "qs")], 8: [a_job(1, "v", x1)], 11: [a_job(1, "qs")]}
        return jobs

    segment(2, 8, {})
    segment(8, 10, {})
    segment(10, 14, four(lambda q: wq_job(10, q)))
    segment(14, 16, four(lambda q: awq_job(14, q)))
    segment(16, 18, {})
    segment(18, 22, four(lambda q: wuk_job(18, q)))
    segment(22, 32, four(lambda q: bqk_job(lambda j: 4 * (j - 22) + q)))
    segment(32, 35, four(lambda q: bqk_job(lambda j: 4 * (j - 22) + q)))
    segment(35, 41, with_a(bqk_job(lambda j: 52 + 2 * (j - 35)), bqk_job(lambda j: 53 + 2 * (j - 35))))
    run_job(bmax_job, 41)
    segment(41, 73, with_a(bpv_job(lambda j: 2 * (j - 41)), bpv_job(lambda j: 2 * (j - 41) + 1)))
    run_job(bfin_job, 73)
    segment(73, 77, with_a(wuv_job(73, 0), wuv_job(73, 1)))
    segment(77, 81, with_a(wuv_job(77, 2), wuv_job(77, 3)))
    segment(81, 96, with_a())
    segment(96, 99, with_a())
    segment(99, 100, {1: [a_job(0, "sv")], 4: [a_job(1, "v")], 7: [proj_job(1, 3)], 10: [proj_job(0, 3)]})
    segment(100, 104, {3: [proj_job(1, 3)], 8: [proj_job(0, 3)]})
    segment(104, 105, {3: [proj_job(1, 3)], 8: [proj_job(0, 3)]})

    last = [(1, mat_unit(7, 0)), (1, mat_unit(7, 1)), (0, mat_unit(7, 0)), (0, mat_unit(7, 1))]

    def tail_job(j):
        for side in range(2):
            out_s[side] += sum(proj(sd, i, (0,)) for sd, i in last if sd == side)

    for t in range(8):
        wait_tick(4, NIT - 1, t)
        if t in (0, 3):
            run_job(proj_job(0 if t else 1, 3), NIT + 1)
    run_job(tail_job, NIT + 1)
    outs = [out_s[0], out_s[1]]
    for t in range(8, 12):
        wait_tick(4, NIT - 1, t)
        if compute:
            side, i = last[t - 8]
            outs[side] = outs[side] + proj(side, i, (1,))
    res = jnp.concatenate(outs, axis=1)
    out_ref[...] = res[:NB, :].astype(out_ref.dtype)


def _build():
    vm = pltpu.VMEM
    scratch = [
        vm((2, NB, DM), BF),
        vm((KV_SLOTS, WIN, DH), BF),
        vm((KV_SLOTS, WIN, DH), BF),
        vm((DM, NH * DH), BF),
        vm((16, 256, DM), BF),
        vm((64, 256, DM), BF),
        vm((DM * NH, DH), BF),
        vm((DM * NH, DH), BF),
        vm((DM * NH, DH), BF),
        vm((16, 256, DM), BF),
        vm((2, 4, 8, 128), BF),
        vm((NH, 8, DH), F32),
        vm((NH * 8, 128), F32),
        vm((NB, 4, NH, 128), BF),
        vm((64, NH, 256), F32),
        vm((NB, NH, 128), F32),
        vm((NB, NH, 128), F32),
        vm((NB, NH, DM), F32),
        vm((4, 8 * NH, 128), F32),
        vm((NH, 8, DH), F32),
        vm((2, 8, 2048), F32),
        vm((NH, 8, DH), BF),
        vm((2, 8, WIN), F32),
        vm((2, 8, DH), F32),
        vm((2, 8, WIN), BF),
        vm((2, 8, DH), F32),
        vm((NH, 8, DH), F32),
        vm((2, 8, DM), F32),
        pltpu.SMEM((1,), jnp.int32),
        pltpu.SemaphoreType.DMA((64,)),
        pltpu.SemaphoreType.DMA((4,)),
        pltpu.SemaphoreType.DMA((2,)),
    ]
    return pl.pallas_call(
        _kernel,
        out_shape=jax.ShapeDtypeStruct((NB, 2 * DM), BF),
        in_specs=[pl.BlockSpec(memory_space=pl.ANY)] * 11,
        out_specs=pl.BlockSpec(memory_space=pltpu.VMEM),
        scratch_shapes=scratch,
        compiler_params=pltpu.CompilerParams(
            vmem_limit_bytes=72 * 1024 * 1024,
            disable_bounds_checks=CFG.get("fast", True),
            disable_semaphore_checks=CFG.get("fast", True),
        ),
    )


def _run(A_x, A_k_cache, A_v_cache, A_wq, A_wo, B_x, B_c_kv, B_w_q, B_w_uk, B_w_uv, B_w_o):
    out = _build()(
        A_x.reshape(NB, DM),
        A_k_cache.reshape(NB * NH, SK, DH),
        A_v_cache.reshape(NB * NH, SK, DH),
        A_wq,
        A_wo.reshape(16, 256, DM),
        B_x.reshape(NB, DM),
        B_c_kv.reshape(64, 256, DM),
        B_w_q.reshape(DM * NH, DH),
        B_w_uk.reshape(DM * NH, DH),
        B_w_uv.reshape(DM * NH, DH),
        B_w_o.reshape(16, 256, DM),
    )
    return out.reshape(NB, 1, 2 * DM)


@jax.jit
def pallas_concat_heads__sliding_block_cached__compressed_kv_cla__decode_kernel(
    A_x: jax.Array,
    A_k_cache: jax.Array,
    A_v_cache: jax.Array,
    A_wq: jax.Array,
    A_wo: jax.Array,
    B_x: jax.Array,
    B_c_kv: jax.Array,
    B_w_q: jax.Array,
    B_w_uk: jax.Array,
    B_w_uv: jax.Array,
    B_w_o: jax.Array,
):
    return _run(A_x, A_k_cache, A_v_cache, A_wq, A_wo, B_x, B_c_kv, B_w_q, B_w_uk, B_w_uv, B_w_o)
```

```python
import functools

import jax
import jax.numpy as jnp
from jax import lax
from jax.experimental import pallas as pl
from jax.experimental.pallas import tpu as pltpu

BF = jnp.bfloat16
F32 = jnp.float32
U32 = jnp.uint32

NB = 4
NH = 32
DH = 128
SK = 4096
WIN = 1024
DM = 512
SCALE = float(DH) ** -0.5

KV_SLOTS = 16
LAG = 2

CUT_A = 15
CUT_B = 17

_NT = (((1,), (1,)), ((), ()))

CFG = dict(compute=True, wide="rows", fence=False, amode="six", off=2)


def _split_pair(w):
    lo = pltpu.bitcast(w << 16, F32).astype(BF)
    hi = pltpu.bitcast(w & U32(0xFFFF0000), F32).astype(BF)
    return lo, hi


def _tile_runs(t0, t1, per_row):
    runs = []
    while t0 < t1:
        r, c = divmod(t0, per_row)
        if c == 0 and t1 - t0 >= per_row:
            n = (t1 - t0) // per_row
            runs.append((r, n, 0, per_row))
            t0 += n * per_row
        else:
            n = min(per_row - c, t1 - t0)
            runs.append((r, 1, c, n))
            t0 += n
    return runs


def _unit_pieces(cut, per_row):
    if CFG["wide"] == "rows" and 1 < per_row < 32:
        cut = (cut + per_row // 2) // per_row * per_row
    lo = [_tile_runs(cut + 32 * p, cut + 32 * (p + 1), per_row) for p in range(3)]
    unit = per_row if per_row < 32 else 1
    mid = ((cut + 96 + 128) // 2 + unit - 1) // unit * unit
    hi = [_tile_runs(0, cut, per_row), _tile_runs(cut + 96, mid, per_row), _tile_runs(mid, 128, per_row)]
    return lo, hi


def _kernel(ax_hbm, k_hbm, v_hbm, awq_hbm, awo_hbm,
            bx_hbm, c_hbm, bwq_hbm, bwuk_hbm, bwuv_hbm, bwo_hbm,
            out_ref,
            x_v, kbuf, vbuf, awq_v, awo_v, c_v, w_v, w32_s, bwo_v,
            x8_s, qb_s, qabs_s, qabs_b, s_s, m_s, l_s, acc_s, cx_s, ctx_s,
            qa_s, qa_b, sa_s, ma_s, p_s, la_s, o_s, out_s, one_s,
            lo_sems, hi_sems, xsems):
    compute = CFG["compute"]

    def mat_unit(it, u):
        return 2 * ((it & 3) + 4 * (u & 1)) + (it >> 2)

    def aligned(x, m):
        return x if isinstance(x, int) else pl.multiple_of(x, m)

    def lead(hbm, vmem, cut, per_row, src_row0=0):
        def rect(si, di, run):
            r, n, c, m = run
            cols = pl.ds(c * 128, m * 128)
            return (hbm.at[si, pl.ds(src_row0 + 8 * r, 8 * n), cols],
                    vmem.at[di, pl.ds(8 * r, 8 * n), cols])
        return rect, _unit_pieces(cut, per_row)

    def flat(hbm, vmem, cut, per_row):
        rows = 8 * 128 // per_row

        def rect(si, di, run):
            r, n, c, m = run
            rs = pl.ds(aligned(si * rows + 8 * r, 8), 8 * n)
            cols = pl.ds(c * 128, m * 128)
            return hbm.at[rs, cols], vmem.at[rs, cols]
        return rect, _unit_pieces(cut, per_row)

    arr = dict(
        bwq=flat(bwq_hbm, w_v.at[0], CUT_B, 1),
        bwuk=flat(bwuk_hbm, w_v.at[1], CUT_B, 1),
        bwuv=flat(bwuv_hbm, w_v.at[2], CUT_B, 1),
        awq=flat(awq_hbm, awq_v, CUT_A, 32),
        c=lead(c_hbm, c_v, CUT_B, 4),
        bwo=lead(bwo_hbm, bwo_v, CUT_B, 4),
        awo=lead(awo_hbm, awo_v, CUT_A, 4),
        k=lead(k_hbm, kbuf, CUT_A, 1, SK - WIN),
        v=lead(v_hbm, vbuf, CUT_A, 1, SK - WIN),
    )

    def pair_phase(a, b):
        def unit(it, u):
            i = mat_unit(it, u)
            return (a if u < 2 else b), i, i
        return unit

    def c_phase(it, u):
        i = 16 * u + 2 * (it & 7) + (it >> 3)
        return "c", i, i

    def kv_phase(it, u):
        g = 2 * it + (u >> 1)
        return ("v" if u & 1 else "k"), g, g & (KV_SLOTS - 1)

    phases = [(0, 8, pair_phase("bwq", "bwuk")),
              (8, 8, pair_phase("awq", "bwuv")),
              (16, 16, c_phase),
              (32, 64, kv_phase),
              (96, 8, pair_phase("bwo", "awo"))]
    NIT = 104

    def phase_of(j):
        for n, (j0, cnt, _) in enumerate(phases):
            if j0 <= j < j0 + cnt:
                return n
        return None

    def copies(ph, j, t, high):
        j0, _, unit = phases[ph]
        name, si, di = unit(j - j0, (t + 2) % 4 if high else t % 4)
        rect, pieces = arr[name]
        sem = hi_sems.at[j & 3] if high else lo_sems.at[(j & 3) * 16 + t]
        out = []
        for run in pieces[1 if high else 0][t // 4]:
            src, dst = rect(si, di, run)
            out.append(pltpu.make_async_copy(src, dst, sem))
        return out

    def start_tick(ph, j, t):
        for cp in copies(ph, j, t, True):
            cp.start(priority=0)
        for cp in copies(ph, j, t, False):
            cp.start(priority=1)

    def wait_tick(ph, j, t):
        if t == 0:
            for tt in range(12):
                for cp in copies(ph, j, tt, True):
                    cp.wait()
        for cp in copies(ph, j, t, False):
            cp.wait()

    def run_job(job, j):
        name = getattr(job, "__qualname__", "job").split(".")[-3 if job.__name__ == "job" else -1]
        if (not compute and "init" not in name) or name in CFG.get("skip", ()):
            return
        if CFG.get("scopes") == "job":
            with jax.named_scope(name):
                job(j)
        elif CFG["fence"]:
            pl.when(one_s[0] > 0)(lambda: job(j))
        else:
            job(j)

    def iteration(j, sph, wphs, jobs):
        for t in range(12):
            if len(wphs) == 1:
                wait_tick(wphs[0], j - LAG, t)
            elif len(wphs) == 2:
                edge = phases[wphs[1]][0] + LAG
                pl.when(j < edge)(lambda: wait_tick(wphs[0], j - LAG, t))
                pl.when(j >= edge)(lambda: wait_tick(wphs[1], j - LAG, t))
            if sph is not None:
                start_tick(sph, j, t)
            for job in jobs.get(t, ()):
                run_job(job, j)

    def segment(j0, j1, jobs):
        sph = phase_of(j0)
        assert all(phase_of(j) == sph for j in range(j0, j1))
        wphs = sorted({phase_of(j - LAG) for j in range(j0, j1) if j >= LAG})
        if CFG.get("scopes") == "seg":
            with jax.named_scope(f"seg{j0:03d}_{j1 - j0}"):
                _segment(j0, j1, sph, wphs, jobs)
        else:
            _segment(j0, j1, sph, wphs, jobs)

    def _segment(j0, j1, sph, wphs, jobs):
        if j1 - j0 == 1:
            iteration(j0, sph, wphs, jobs)
        else:
            def body(j, carry):
                iteration(j, sph, wphs, jobs)
                return carry
            lax.fori_loop(j0, j1, body, 0)

    def repack_job(index):
        def job(j):
            mat, ch = index(j)
            w = w_v[mat, pl.ds(aligned(ch * 4096, 4096), 4096), :]
            w32_s[mat, ch] = pltpu.bitcast(w, U32)
        return job

    def head_pair(mat, ch, hp):
        return _split_pair(w32_s[mat, ch, pl.ds(hp, 128, stride=16), :])

    def wq_job(j0, q):
        def job(j):
            ch = j - j0
            x = x8_s[1, ch]
            for hp in range(4 * q, 4 * q + 4):
                lo, hi = head_pair(0, ch, hp)
                qb_s[2 * hp] += jnp.dot(x, lo, preferred_element_type=F32)
                qb_s[2 * hp + 1] += jnp.dot(x, hi, preferred_element_type=F32)
        return job

    def awq_job(j0, q):
        def job(j):
            half = j - j0
            cols = pl.ds(aligned(half * 2048, 2048), 2048)
            qa_s[half] += jnp.dot(x8_s[0, q], awq_v[pl.ds(q * 128, 128), cols],
                                  preferred_element_type=F32)
            if q == 3:
                for hh in range(16):
                    qa_b[half * 16 + hh] = qa_s[half, :, hh * 128:(hh + 1) * 128].astype(BF)
        return job

    def wuk_job(j0, q):
        def job(j):
            ch = j - j0
            for hp in range(4 * q, 4 * q + 4):
                lo, hi = head_pair(1, ch, hp)
                for h, w in ((2 * hp, lo), (2 * hp + 1, hi)):
                    qabs_s[pl.ds(8 * h, 8), :] = lax.dot_general(
                        qb_s[h].astype(BF), w, _NT, preferred_element_type=F32)
            if q == 3:
                for b in range(NB):
                    qabs_b[b, ch] = qabs_s[pl.ds(b, NH, stride=8), :].astype(BF)
        return job

    def bqk_job(index):
        def job(j):
            n = index(j)
            b = n & 3
            k = n >> 2
            i = 16 * b + 2 * (k & 7) + (k >> 3)
            q = jnp.concatenate([qabs_b[b, ch] for ch in range(4)], axis=1)
            s = lax.dot_general(q, c_v[i], _NT, preferred_element_type=F32)
            s_s[i] = s
            m_s[b] = jnp.maximum(m_s[b], jnp.maximum(s[:, :128], s[:, 128:]))
        return job

    def bmax_job(j):
        for b in range(NB):
            m_s[b] = jnp.broadcast_to(jnp.max(m_s[b], axis=-1, keepdims=True), (NH, 128))

    def bpv_job(index):
        def job(j):
            i = index(j)
            b = i >> 4
            m = m_s[b]
            s = s_s[i]
            p0 = jnp.exp((s[:, :128] - m) * SCALE)
            p1 = jnp.exp((s[:, 128:] - m) * SCALE)
            l_s[b] += p0 + p1
            p = jnp.concatenate([p0, p1], axis=1).astype(BF)
            acc_s[b] += jnp.dot(p, c_v[i], preferred_element_type=F32)
        return job

    def bfin_job(j):
        for b in range(NB):
            ctxc = acc_s[b] * (1.0 / jnp.sum(l_s[b], axis=-1, keepdims=True))
            for ch in range(4):
                cx_s[ch, pl.ds(b * NH, NH), :] = ctxc[:, ch * 128:(ch + 1) * 128]

    def wuv_job(j0, q):
        def job(j):
            ch = j - j0
            for hp in range(4 * q, 4 * q + 4):
                lo, hi = head_pair(2, ch, hp)
                for h, w in ((2 * hp, lo), (2 * hp + 1, hi)):
                    lhs = cx_s[ch, pl.ds(h, 8, stride=NH), :].astype(BF)
                    ctx_s[h] += jnp.dot(lhs, w, preferred_element_type=F32)
        return job

    row = lax.broadcasted_iota(jnp.int32, (8, DH), 0)

    def a_scores(g, e):
        s = lax.dot_general(qa_b[g & (NH - 1)], kbuf[g & (KV_SLOTS - 1)], _NT,
                            preferred_element_type=F32)
        sa_s[e] = s
        parts = [s[:, c * 128:(c + 1) * 128] for c in range(8)]
        while len(parts) > 1:
            parts = [jnp.maximum(parts[2 * c], parts[2 * c + 1]) for c in range(len(parts) // 2)]
        ma_s[e] = parts[0]

    def a_softmax(e):
        m = jnp.max(ma_s[e], axis=-1, keepdims=True)
        p = jnp.exp((sa_s[e] - m) * SCALE)
        p_s[e] = p.astype(BF)
        parts = [p[:, c * 128:(c + 1) * 128] for c in range(8)]
        while len(parts) > 1:
            parts = [parts[2 * c] + parts[2 * c + 1] for c in range(len(parts) // 2)]
        la_s[e] = parts[0]

    def a_values(g, e):
        o = jnp.dot(p_s[e], vbuf[g & (KV_SLOTS - 1)], preferred_element_type=F32)
        inv = 1.0 / jnp.sum(la_s[e], axis=-1, keepdims=True)
        h = g & (NH - 1)
        o_s[h] = jnp.where(row == (g >> 5), o * inv, o_s[h])

    def a_job(e, stages="qsv", also=None):
        def job(j):
            g = 2 * (j - 35) + e
            if "v" in stages:
                a_values(g - 2, e)
            if also is not None:
                also(j)
            if "q" in stages:
                a_scores(g, e)
            if "s" in stages:
                a_softmax(1 - e)
        return job

    def proj(side, i, halves=(0, 1)):
        w_v, src = ((awo_v, o_s), (bwo_v, ctx_s))[side]
        acc = None
        for hf in halves:
            d = jnp.dot(src[2 * i + hf].astype(BF), w_v[i, pl.ds(hf * 128, 128), :],
                        preferred_element_type=F32)
            acc = d if acc is None else acc + d
        return acc

    def proj_job(side, lag):
        def job(j):
            it = j - lag - 96
            out_s[side] += proj(side, mat_unit(it, 0)) + proj(side, mat_unit(it, 1))
        return job

    cxa = pltpu.make_async_copy(ax_hbm, x_v.at[0], xsems.at[0])
    cxb = pltpu.make_async_copy(bx_hbm, x_v.at[1], xsems.at[1])
    for j in range(LAG):
        for t in range(12):
            start_tick(0, j, t)
    cxa.start()
    cxb.start()
    one_s[0] = 1

    def init_job(j):
        for r in (qb_s, qa_s, l_s, acc_s, cx_s, ctx_s, sa_s, ma_s, p_s, o_s, out_s):
            r[...] = jnp.zeros_like(r)
        la_s[...] = jnp.ones_like(la_s)
        m_s[...] = jnp.full(m_s.shape, -jnp.inf, F32)

    def vinit_job(j):
        vbuf[KV_SLOTS - 2 + j - 8] = jnp.zeros((WIN, DH), BF)

    def x_job(j):
        for t in range(2):
            x8 = jnp.concatenate([x_v[t].astype(F32), jnp.zeros((8 - NB, DM), F32)], axis=0)
            for ch in range(4):
                x8_s[t, ch] = x8[:, ch * 128:(ch + 1) * 128].astype(BF)

    def four(mk):
        return {3 * q + CFG['off']: [mk(q)] for q in range(4)}

    def with_a(x0=None, x1=None):
        mode = CFG.get("amode", "merged")
        if mode == "merged":
            jobs = {2: [a_job(0)], 8: [a_job(1)]}
            if x0 is not None:
                jobs[5] = [x0]
                jobs[11] = [x1]
        else:
            o = CFG["off"]
            if mode == "split":
                jobs = {o: [a_job(0, "v", x0)], 3 + o: [a_job(0, "qs")], 6 + o: [a_job(1, "v", x1)], 9 + o: [a_job(1, "qs")]}
            elif mode == "split2":
                jobs = {o: [a_job(0, "vs", x0)], 3 + o: [a_job(0, "q")], 6 + o: [a_job(1, "vs", x1)], 9 + o: [a_job(1, "q")]}
            elif mode == "six":
                jobs = {0: [a_job(0, "v")], 2: [a_job(0, "qs")], 6: [a_job(1, "v")], 8: [a_job(1, "qs")]}
                if x0 is not None:
                    jobs[4] = [x0]
                    jobs[10] = [x1]
        return jobs

    segment(2, 8, {})
    cxa.wait()
    cxb.wait()
    x_job(8)
    init_job(8)
    segment(8, 10, {5: [vinit_job]})
    segment(10, 12, four(lambda q: repack_job(lambda j: (j - 10, q))))
    segment(12, 16, four(lambda q: wq_job(12, q)))
    segment(16, 20, four(lambda q: wuk_job(16, q)))
    segment(20, 22, four(lambda q: awq_job(20, q)))
    segment(22, 32, four(lambda q: bqk_job(lambda j: 4 * (j - 22) + q)))
    segment(32, 35, four(lambda q: bqk_job(lambda j: 4 * (j - 22) + q)))
    segment(35, 41, with_a(bqk_job(lambda j: 52 + 2 * (j - 35)), bqk_job(lambda j: 53 + 2 * (j - 35))))
    run_job(bmax_job, 41)
    segment(41, 73, with_a(bpv_job(lambda j: 2 * (j - 41)), bpv_job(lambda j: 2 * (j - 41) + 1)))
    run_job(bfin_job, 73)
    segment(73, 75, with_a(repack_job(lambda j: (2, 2 * (j - 73))), repack_job(lambda j: (2, 2 * (j - 73) + 1))))
    segment(75, 79, with_a(wuv_job(75, 0), wuv_job(75, 1)))
    segment(79, 83, with_a(wuv_job(79, 2), wuv_job(79, 3)))
    segment(83, 96, with_a())
    segment(96, 99, with_a())
    segment(99, 100, {1: [a_job(0, "sv")], 4: [a_job(1, "v")], 7: [proj_job(1, 3)], 10: [proj_job(0, 3)]})
    segment(100, 104, {3: [proj_job(1, 3)], 8: [proj_job(0, 3)]})
    segment(104, 105, {3: [proj_job(1, 3)], 8: [proj_job(0, 3)]})

    def half_job(side, hf):
        def job(j):
            out_s[side] += proj(side, mat_unit(7, 0), (hf,)) + proj(side, mat_unit(7, 1), (hf,))
        return job

    tail = {0: proj_job(1, 3), 2: proj_job(0, 3), 5: half_job(1, 0), 7: half_job(0, 0), 9: half_job(1, 1)}
    for t in range(12):
        wait_tick(4, NIT - 1, t)
        if t in tail:
            run_job(tail[t], NIT + 1)
    outs = [out_s[0], out_s[1]]
    if compute:
        outs[0] = outs[0] + proj(0, mat_unit(7, 0), (1,)) + proj(0, mat_unit(7, 1), (1,))
    res = jnp.concatenate(outs, axis=1)
    out_ref[...] = res[:NB, :].astype(out_ref.dtype)


def _build():
    vm = pltpu.VMEM
    scratch = [
        vm((2, NB, DM), BF),
        vm((KV_SLOTS, WIN, DH), BF),
        vm((KV_SLOTS, WIN, DH), BF),
        vm((DM, NH * DH), BF),
        vm((16, 256, DM), BF),
        vm((64, 256, DM), BF),
        vm((3, DM * NH, DH), BF),
        vm((3, 4, 2048, DH), U32),
        vm((16, 256, DM), BF),
        vm((2, 4, 8, 128), BF),
        vm((NH, 8, DH), F32),
        vm((NH * 8, 128), F32),
        vm((NB, 4, NH, 128), BF),
        vm((64, NH, 256), F32),
        vm((NB, NH, 128), F32),
        vm((NB, NH, 128), F32),
        vm((NB, NH, DM), F32),
        vm((4, 8 * NH, 128), F32),
        vm((NH, 8, DH), F32),
        vm((2, 8, 2048), F32),
        vm((NH, 8, DH), BF),
        vm((2, 8, WIN), F32),
        vm((2, 8, DH), F32),
        vm((2, 8, WIN), BF),
        vm((2, 8, DH), F32),
        vm((NH, 8, DH), F32),
        vm((2, 8, DM), F32),
        pltpu.SMEM((1,), jnp.int32),
        pltpu.SemaphoreType.DMA((64,)),
        pltpu.SemaphoreType.DMA((4,)),
        pltpu.SemaphoreType.DMA((2,)),
    ]
    return pl.pallas_call(
        _kernel,
        out_shape=jax.ShapeDtypeStruct((NB, 2 * DM), BF),
        in_specs=[pl.BlockSpec(memory_space=pl.ANY)] * 11,
        out_specs=pl.BlockSpec(memory_space=pltpu.VMEM),
        scratch_shapes=scratch,
        compiler_params=pltpu.CompilerParams(
            vmem_limit_bytes=80 * 1024 * 1024,
            disable_bounds_checks=CFG.get("fast", True),
            disable_semaphore_checks=CFG.get("fast", True),
        ),
    )


def _run(A_x, A_k_cache, A_v_cache, A_wq, A_wo, B_x, B_c_kv, B_w_q, B_w_uk, B_w_uv, B_w_o):
    out = _build()(
        A_x.reshape(NB, DM),
        A_k_cache.reshape(NB * NH, SK, DH),
        A_v_cache.reshape(NB * NH, SK, DH),
        A_wq,
        A_wo.reshape(16, 256, DM),
        B_x.reshape(NB, DM),
        B_c_kv.reshape(64, 256, DM),
        B_w_q.reshape(DM * NH, DH),
        B_w_uk.reshape(DM * NH, DH),
        B_w_uv.reshape(DM * NH, DH),
        B_w_o.reshape(16, 256, DM),
    )
    return out.reshape(NB, 1, 2 * DM)


@jax.jit
def pallas_concat_heads__sliding_block_cached__compressed_kv_cla__decode_kernel(
    A_x: jax.Array,
    A_k_cache: jax.Array,
    A_v_cache: jax.Array,
    A_wq: jax.Array,
    A_wo: jax.Array,
    B_x: jax.Array,
    B_c_kv: jax.Array,
    B_w_q: jax.Array,
    B_w_uk: jax.Array,
    B_w_uv: jax.Array,
    B_w_o: jax.Array,
):
    return _run(A_x, A_k_cache, A_v_cache, A_wq, A_wo, B_x, B_c_kv, B_w_q, B_w_uk, B_w_uv, B_w_o)
```

```python
import jax
import jax.numpy as jnp
from jax import lax
from jax.experimental import pallas as pl
from jax.experimental.pallas import tpu as pltpu

BF = jnp.bfloat16
F32 = jnp.float32
U32 = jnp.uint32

NB = 4
NH = 32
DH = 128
SK = 4096
WIN = 1024
DM = 512
SCALE = float(DH) ** -0.5

KV_SLOTS = 16
LAG = 2
TICKS = 12
NIT = 104

CUT_A = 15
CUT_B = 17

_NT = (((1,), (1,)), ((), ()))


def _split_pair(w):
    lo = pltpu.bitcast(w << 16, F32).astype(BF)
    hi = pltpu.bitcast(w & U32(0xFFFF0000), F32).astype(BF)
    return lo, hi


def _tree(op, parts):
    while len(parts) > 1:
        parts = [op(parts[2 * c], parts[2 * c + 1]) for c in range(len(parts) // 2)]
    return parts[0]


def _tile_runs(t0, t1, per_row):
    runs = []
    while t0 < t1:
        r, c = divmod(t0, per_row)
        if c == 0 and t1 - t0 >= per_row:
            n = (t1 - t0) // per_row
            runs.append((r, n, 0, per_row))
            t0 += n * per_row
        else:
            n = min(per_row - c, t1 - t0)
            runs.append((r, 1, c, n))
            t0 += n
    return runs


def _unit_pieces(cut, per_row):
    step = per_row if per_row < 32 else 1
    cut = (cut + step // 2) // step * step
    mid = ((cut + 96 + 128) // 2 + step - 1) // step * step
    lo = [_tile_runs(cut + 32 * p, cut + 32 * (p + 1), per_row) for p in range(3)]
    hi = [_tile_runs(0, cut, per_row), _tile_runs(cut + 96, mid, per_row), _tile_runs(mid, 128, per_row)]
    return lo, hi


def _aligned(x, m):
    return x if isinstance(x, int) else pl.multiple_of(x, m)


def _kernel(ax_hbm, k_hbm, v_hbm, awq_hbm, awo_hbm,
            bx_hbm, c_hbm, bwq_hbm, bwuk_hbm, bwuv_hbm, bwo_hbm,
            out_ref,
            x_v, kbuf, vbuf, awq_v, awo_v, c_v, w_v, w32_s, bwo_v,
            x8_s, qb_s, qabs_s, qabs_b, s_s, m_s, l_s, acc_s, cx_s, ctx_s,
            qa_s, qa_b, sa_s, ma_s, p_s, la_s, o_s, out_s,
            lo_sems, hi_sems, x_sems):

    def lead(hbm, vmem, cut, per_row, src_row0=0):
        def rect(si, di, run):
            r, n, c, m = run
            cols = pl.ds(c * 128, m * 128)
            return (hbm.at[si, pl.ds(src_row0 + 8 * r, 8 * n), cols],
                    vmem.at[di, pl.ds(8 * r, 8 * n), cols])
        return rect, _unit_pieces(cut, per_row)

    def flat(hbm, vmem, cut, per_row):
        rows = 8 * 128 // per_row

        def rect(si, di, run):
            r, n, c, m = run
            rs = pl.ds(_aligned(si * rows + 8 * r, 8), 8 * n)
            cols = pl.ds(c * 128, m * 128)
            return hbm.at[rs, cols], vmem.at[rs, cols]
        return rect, _unit_pieces(cut, per_row)

    arrays = dict(
        bwq=flat(bwq_hbm, w_v.at[0], CUT_B, 1),
        bwuk=flat(bwuk_hbm, w_v.at[1], CUT_B, 1),
        bwuv=flat(bwuv_hbm, w_v.at[2], CUT_B, 1),
        awq=flat(awq_hbm, awq_v, CUT_A, 32),
        c=lead(c_hbm, c_v, CUT_B, 4),
        bwo=lead(bwo_hbm, bwo_v, CUT_B, 4),
        awo=lead(awo_hbm, awo_v, CUT_A, 4),
        k=lead(k_hbm, kbuf, CUT_A, 1, SK - WIN),
        v=lead(v_hbm, vbuf, CUT_A, 1, SK - WIN),
    )

    def mat_unit(it, u):
        return 2 * ((it & 3) + 4 * (u & 1)) + (it >> 2)

    def c_unit(b, it):
        return 16 * b + 2 * (it & 7) + (it >> 3)

    def pair_phase(a, b):
        def unit(it, u):
            i = mat_unit(it, u)
            return (a if u < 2 else b), i, i
        return unit

    def c_phase(it, u):
        i = c_unit(u, it)
        return "c", i, i

    def kv_phase(it, u):
        g = 2 * it + (u >> 1)
        return ("v" if u & 1 else "k"), g, g & (KV_SLOTS - 1)

    phases = [(0, 8, pair_phase("bwq", "bwuk")),
              (8, 8, pair_phase("awq", "bwuv")),
              (16, 16, c_phase),
              (32, 64, kv_phase),
              (96, 8, pair_phase("bwo", "awo"))]

    def phase_of(j):
        for n, (j0, cnt, _) in enumerate(phases):
            if j0 <= j < j0 + cnt:
                return n
        return None

    def copies(ph, j, t, high):
        j0, _, unit = phases[ph]
        name, si, di = unit(j - j0, (t + 2) % 4 if high else t % 4)
        rect, pieces = arrays[name]
        sem = hi_sems.at[j & 3] if high else lo_sems.at[(j & 3) * 16 + t]
        return [pltpu.make_async_copy(*rect(si, di, run), sem)
                for run in pieces[1 if high else 0][t // 4]]

    def start_tick(ph, j, t):
        for cp in copies(ph, j, t, True):
            cp.start(priority=0)
        for cp in copies(ph, j, t, False):
            cp.start(priority=1)

    def wait_tick(ph, j, t):
        if t == 0:
            for tt in range(TICKS):
                for cp in copies(ph, j, tt, True):
                    cp.wait()
        for cp in copies(ph, j, t, False):
            cp.wait()

    def segment(j0, j1, jobs):
        sph = phase_of(j0)
        assert all(phase_of(j) == sph for j in range(j0, j1))
        wphs = sorted({phase_of(j - LAG) for j in range(j0, j1)})

        def iteration(j):
            for t in range(TICKS):
                if len(wphs) == 1:
                    wait_tick(wphs[0], j - LAG, t)
                else:
                    edge = phases[wphs[1]][0] + LAG
                    pl.when(j < edge)(lambda: wait_tick(wphs[0], j - LAG, t))
                    pl.when(j >= edge)(lambda: wait_tick(wphs[1], j - LAG, t))
                if sph is not None:
                    start_tick(sph, j, t)
                if t in jobs:
                    jobs[t](j)

        if j1 - j0 == 1:
            iteration(j0)
        else:
            def body(j, carry):
                iteration(j)
                return carry
            lax.fori_loop(j0, j1, body, 0)

    def repack_job(index):
        def job(j):
            mat, ch = index(j)
            w = w_v[mat, pl.ds(_aligned(ch * 4096, 4096), 4096), :]
            w32_s[mat, ch] = pltpu.bitcast(w, U32)
        return job

    def heads(mat, ch, q):
        for hp in range(4 * q, 4 * q + 4):
            lo, hi = _split_pair(w32_s[mat, ch, pl.ds(hp, 128, stride=16), :])
            yield 2 * hp, lo
            yield 2 * hp + 1, hi

    def wq_job(j0, q):
        def job(j):
            x = x8_s[1, j - j0]
            for h, w in heads(0, j - j0, q):
                qb_s[h] += jnp.dot(x, w, preferred_element_type=F32)
        return job

    def wuk_job(j0, q):
        def job(j):
            for h, w in heads(1, j - j0, q):
                qabs_s[pl.ds(8 * h, 8), :] = lax.dot_general(
                    qb_s[h].astype(BF), w, _NT, preferred_element_type=F32)
            if q == 3:
                for b in range(NB):
                    qabs_b[b, j - j0] = qabs_s[pl.ds(b, NH, stride=8), :].astype(BF)
        return job

    def bqk_job(index):
        def job(j):
            n = index(j)
            b = n & 3
            i = c_unit(b, n >> 2)
            q = jnp.concatenate([qabs_b[b, ch] for ch in range(4)], axis=1)
            s = lax.dot_general(q, c_v[i], _NT, preferred_element_type=F32)
            s_s[i] = s
            m_s[b] = jnp.maximum(m_s[b], jnp.maximum(s[:, :128], s[:, 128:]))
        return job

    def bmax_job():
        for b in range(NB):
            m_s[b] = jnp.broadcast_to(jnp.max(m_s[b], axis=-1, keepdims=True), (NH, 128))

    def bpv_job(index):
        def job(j):
            i = index(j)
            b = i >> 4
            m = m_s[b]
            s = s_s[i]
            p0 = jnp.exp((s[:, :128] - m) * SCALE)
            p1 = jnp.exp((s[:, 128:] - m) * SCALE)
            l_s[b] += p0 + p1
            p = jnp.concatenate([p0, p1], axis=1).astype(BF)
            acc_s[b] += jnp.dot(p, c_v[i], preferred_element_type=F32)
        return job

    def bnorm_job():
        for b in range(NB):
            ctxc = acc_s[b] * (1.0 / jnp.sum(l_s[b], axis=-1, keepdims=True))
            for ch in range(4):
                cx_s[ch, pl.ds(b * NH, NH), :] = ctxc[:, ch * 128:(ch + 1) * 128]

    def wuv_job(j0, q):
        def job(j):
            for h, w in heads(2, j - j0, q):
                lhs = cx_s[j - j0, pl.ds(h, 8, stride=NH), :].astype(BF)
                ctx_s[h] += jnp.dot(lhs, w, preferred_element_type=F32)
        return job

    def awq_job(j0, q):
        def job(j):
            half = j - j0
            cols = pl.ds(_aligned(half * 2048, 2048), 2048)
            qa_s[half] += jnp.dot(x8_s[0, q], awq_v[pl.ds(q * 128, 128), cols],
                                  preferred_element_type=F32)
            if q == 3:
                for hh in range(16):
                    qa_b[half * 16 + hh] = qa_s[half, :, hh * 128:(hh + 1) * 128].astype(BF)
        return job

    A0 = 35
    row = lax.broadcasted_iota(jnp.int32, (8, DH), 0)

    def lanes(x):
        return [x[:, c * 128:(c + 1) * 128] for c in range(WIN // 128)]

    def a_scores_job(e, scores=True):
        def job(j):
            if scores:
                g = 2 * (j - A0) + e
                s = lax.dot_general(qa_b[g & (NH - 1)], kbuf[g & (KV_SLOTS - 1)], _NT,
                                    preferred_element_type=F32)
                sa_s[e] = s
                ma_s[e] = _tree(jnp.maximum, lanes(s))
            m = jnp.max(ma_s[1 - e], axis=-1, keepdims=True)
            p = jnp.exp((sa_s[1 - e] - m) * SCALE)
            p_s[1 - e] = p.astype(BF)
            la_s[1 - e] = _tree(jnp.add, lanes(p))
        return job

    def a_values_job(e):
        def job(j):
            g = 2 * (j - A0) + e - 2
            o = jnp.dot(p_s[e], vbuf[g & (KV_SLOTS - 1)], preferred_element_type=F32)
            inv = 1.0 / jnp.sum(la_s[e], axis=-1, keepdims=True)
            h = g & (NH - 1)
            o_s[h] = jnp.where(row == (g >> 5), o * inv, o_s[h])
        return job

    def proj(side, i, halves):
        w_ref, src = ((awo_v, o_s), (bwo_v, ctx_s))[side]
        return sum(jnp.dot(src[2 * i + hf].astype(BF), w_ref[i, pl.ds(hf * 128, 128), :],
                           preferred_element_type=F32) for hf in halves)

    def proj_pair(side, it, halves=(0, 1)):
        return proj(side, mat_unit(it, 0), halves) + proj(side, mat_unit(it, 1), halves)

    def proj_job(side):
        def job(j):
            out_s[side] += proj_pair(side, j - 99)
        return job

    def half_job(side, hf):
        def job(j):
            out_s[side] += proj_pair(side, 7, (hf,))
        return job

    def four(mk):
        return {3 * q + 2: mk(q) for q in range(4)}

    def with_a(x0=None, x1=None):
        if x0 is None:
            return {0: a_values_job(0), 3: a_scores_job(0), 6: a_values_job(1), 9: a_scores_job(1)}
        return {0: a_values_job(0), 2: a_scores_job(0), 4: x0,
                6: a_values_job(1), 8: a_scores_job(1), 10: x1}

    def vinit_job(j):
        vbuf[KV_SLOTS - 2 + j - 8] = jnp.zeros((WIN, DH), BF)

    x_copies = [pltpu.make_async_copy(src, x_v.at[n], x_sems.at[n])
                for n, src in enumerate((ax_hbm, bx_hbm))]
    for j in range(LAG):
        for t in range(TICKS):
            start_tick(0, j, t)
    for cp in x_copies:
        cp.start()

    segment(2, 8, {})
    for cp in x_copies:
        cp.wait()
    for n in range(2):
        x8 = jnp.concatenate([x_v[n].astype(F32), jnp.zeros((8 - NB, DM), F32)], axis=0)
        for ch in range(4):
            x8_s[n, ch] = x8[:, ch * 128:(ch + 1) * 128].astype(BF)
    for r in (qb_s, qa_s, l_s, acc_s, cx_s, ctx_s, sa_s, ma_s, p_s, o_s, out_s):
        r[...] = jnp.zeros_like(r)
    la_s[...] = jnp.ones_like(la_s)
    m_s[...] = jnp.full(m_s.shape, -jnp.inf, F32)

    segment(8, 10, {5: vinit_job})
    segment(10, 12, four(lambda q: repack_job(lambda j: (j - 10, q))))
    segment(12, 16, four(lambda q: wq_job(12, q)))
    segment(16, 20, four(lambda q: wuk_job(16, q)))
    segment(20, 22, four(lambda q: awq_job(20, q)))
    segment(22, 32, four(lambda q: bqk_job(lambda j: 4 * (j - 22) + q)))
    segment(32, 35, four(lambda q: bqk_job(lambda j: 4 * (j - 22) + q)))
    segment(35, 41, with_a(bqk_job(lambda j: 52 + 2 * (j - 35)), bqk_job(lambda j: 53 + 2 * (j - 35))))
    bmax_job()
    segment(41, 73, with_a(bpv_job(lambda j: 2 * (j - 41)), bpv_job(lambda j: 2 * (j - 41) + 1)))
    bnorm_job()
    segment(73, 75, with_a(repack_job(lambda j: (2, 2 * (j - 73))),
                           repack_job(lambda j: (2, 2 * (j - 73) + 1))))
    segment(75, 79, with_a(wuv_job(75, 0), wuv_job(75, 1)))
    segment(79, 83, with_a(wuv_job(79, 2), wuv_job(79, 3)))
    segment(83, 96, with_a())
    segment(96, 99, with_a())
    segment(99, 100, {0: a_values_job(0), 2: a_scores_job(0, scores=False), 4: a_values_job(1),
                      7: proj_job(1), 10: proj_job(0)})
    segment(100, 104, {3: proj_job(1), 8: proj_job(0)})
    segment(104, 105, {3: proj_job(1), 8: proj_job(0)})
    segment(105, 106, {0: proj_job(1), 2: proj_job(0), 5: half_job(1, 0), 7: half_job(0, 0),
                       9: half_job(1, 1)})
    res = jnp.concatenate([out_s[0] + proj_pair(0, 7, (1,)), out_s[1]], axis=1)
    out_ref[...] = res[:NB, :].astype(out_ref.dtype)


@jax.jit
def pallas_concat_heads__sliding_block_cached__compressed_kv_cla__decode_kernel(
    A_x: jax.Array,
    A_k_cache: jax.Array,
    A_v_cache: jax.Array,
    A_wq: jax.Array,
    A_wo: jax.Array,
    B_x: jax.Array,
    B_c_kv: jax.Array,
    B_w_q: jax.Array,
    B_w_uk: jax.Array,
    B_w_uv: jax.Array,
    B_w_o: jax.Array,
):
    vm = pltpu.VMEM
    scratch = [
        vm((2, NB, DM), BF),
        vm((KV_SLOTS, WIN, DH), BF),
        vm((KV_SLOTS, WIN, DH), BF),
        vm((DM, NH * DH), BF),
        vm((16, 256, DM), BF),
        vm((64, 256, DM), BF),
        vm((3, DM * NH, DH), BF),
        vm((3, 4, 2048, DH), U32),
        vm((16, 256, DM), BF),
        vm((2, 4, 8, 128), BF),
        vm((NH, 8, DH), F32),
        vm((NH * 8, 128), F32),
        vm((NB, 4, NH, 128), BF),
        vm((64, NH, 256), F32),
        vm((NB, NH, 128), F32),
        vm((NB, NH, 128), F32),
        vm((NB, NH, DM), F32),
        vm((4, 8 * NH, 128), F32),
        vm((NH, 8, DH), F32),
        vm((2, 8, 2048), F32),
        vm((NH, 8, DH), BF),
        vm((2, 8, WIN), F32),
        vm((2, 8, DH), F32),
        vm((2, 8, WIN), BF),
        vm((2, 8, DH), F32),
        vm((NH, 8, DH), F32),
        vm((2, 8, DM), F32),
        pltpu.SemaphoreType.DMA((64,)),
        pltpu.SemaphoreType.DMA((4,)),
        pltpu.SemaphoreType.DMA((2,)),
    ]
    out = pl.pallas_call(
        _kernel,
        out_shape=jax.ShapeDtypeStruct((NB, 2 * DM), BF),
        in_specs=[pl.BlockSpec(memory_space=pl.ANY)] * 11,
        out_specs=pl.BlockSpec(memory_space=pltpu.VMEM),
        scratch_shapes=scratch,
        compiler_params=pltpu.CompilerParams(
            vmem_limit_bytes=80 * 1024 * 1024,
            disable_bounds_checks=True,
            disable_semaphore_checks=True,
        ),
    )(
        A_x.reshape(NB, DM),
        A_k_cache.reshape(NB * NH, SK, DH),
        A_v_cache.reshape(NB * NH, SK, DH),
        A_wq,
        A_wo.reshape(16, 256, DM),
        B_x.reshape(NB, DM),
        B_c_kv.reshape(64, 256, DM),
        B_w_q.reshape(DM * NH, DH),
        B_w_uk.reshape(DM * NH, DH),
        B_w_uv.reshape(DM * NH, DH),
        B_w_o.reshape(16, 256, DM),
    )
    return out.reshape(NB, 1, 2 * DM)
```

```python
import jax
import jax.numpy as jnp
from jax import lax
from jax.experimental import pallas as pl
from jax.experimental.pallas import tpu as pltpu

BF = jnp.bfloat16
F32 = jnp.float32
U32 = jnp.uint32

NB = 4
NH = 32
DH = 128
SK = 4096
WIN = 1024
DM = 512
SCALE = float(DH) ** -0.5

KV_SLOTS = 16
LAG = 2
TICKS = 12
NIT = 104

CUT_A = 15
CUT_B = 17

_NT = (((1,), (1,)), ((), ()))


def _split_pair(w):
    lo = pltpu.bitcast(w << 16, F32).astype(BF)
    hi = pltpu.bitcast(w & U32(0xFFFF0000), F32).astype(BF)
    return lo, hi


def _tree(op, parts):
    while len(parts) > 1:
        parts = [op(parts[2 * c], parts[2 * c + 1]) for c in range(len(parts) // 2)]
    return parts[0]


def _tile_runs(t0, t1, per_row):
    runs = []
    while t0 < t1:
        r, c = divmod(t0, per_row)
        if c == 0 and t1 - t0 >= per_row:
            n = (t1 - t0) // per_row
            runs.append((r, n, 0, per_row))
            t0 += n * per_row
        else:
            n = min(per_row - c, t1 - t0)
            runs.append((r, 1, c, n))
            t0 += n
    return runs


def _unit_pieces(cut, per_row):
    step = per_row if per_row < 32 else 1
    cut = (cut + step // 2) // step * step
    mid = ((cut + 96 + 128) // 2 + step - 1) // step * step
    lo = [_tile_runs(cut + 32 * p, cut + 32 * (p + 1), per_row) for p in range(3)]
    hi = [_tile_runs(0, cut, per_row), _tile_runs(cut + 96, mid, per_row), _tile_runs(mid, 128, per_row)]
    return lo, hi


def _aligned(x, m):
    return x if isinstance(x, int) else pl.multiple_of(x, m)


def _kernel(ax_hbm, k_hbm, v_hbm, awq_hbm, awo_hbm,
            bx_hbm, c_hbm, bwq_hbm, bwuk_hbm, bwuv_hbm, bwo_hbm,
            out_ref,
            x_v, kbuf, vbuf, awq_v, awo_v, c_v, w_v, w32_s, bwo_v,
            x8_s, qb_s, qabs_s, qabs_b, s_s, m_s, l_s, acc_s, cx_s, ctx_s,
            qa_s, qa_b, sa_s, ma_s, p_s, la_s, o_s, out_s,
            lo_sems, hi_sems, x_sems):

    def lead(hbm, vmem, cut, per_row, src_row0=0):
        def rect(si, di, run):
            r, n, c, m = run
            cols = pl.ds(c * 128, m * 128)
            return (hbm.at[si, pl.ds(src_row0 + 8 * r, 8 * n), cols],
                    vmem.at[di, pl.ds(8 * r, 8 * n), cols])
        return rect, _unit_pieces(cut, per_row)

    def flat(hbm, vmem, cut, per_row):
        rows = 8 * 128 // per_row

        def rect(si, di, run):
            r, n, c, m = run
            rs = pl.ds(_aligned(si * rows + 8 * r, 8), 8 * n)
            cols = pl.ds(c * 128, m * 128)
            return hbm.at[rs, cols], vmem.at[rs, cols]
        return rect, _unit_pieces(cut, per_row)

    arrays = dict(
        bwq=flat(bwq_hbm, w_v.at[0], CUT_B, 1),
        bwuk=flat(bwuk_hbm, w_v.at[1], CUT_B, 1),
        bwuv=flat(bwuv_hbm, w_v.at[2], CUT_B, 1),
        awq=flat(awq_hbm, awq_v, CUT_A, 32),
        c=lead(c_hbm, c_v, CUT_B, 4),
        bwo=lead(bwo_hbm, bwo_v, CUT_B, 4),
        awo=lead(awo_hbm, awo_v, CUT_A, 4),
        k=lead(k_hbm, kbuf, CUT_A, 1, SK - WIN),
        v=lead(v_hbm, vbuf, CUT_A, 1, SK - WIN),
    )

    def mat_unit(it, u):
        return 2 * ((it & 3) + 4 * (u & 1)) + (it >> 2)

    def c_unit(b, it):
        return 16 * b + 2 * (it & 7) + (it >> 3)

    def pair_phase(a, b):
        def unit(it, u):
            i = mat_unit(it, u)
            return (a if u < 2 else b), i, i
        return unit

    def c_phase(it, u):
        i = c_unit(u, it)
        return "c", i, i

    def kv_phase(it, u):
        g = 2 * it + (u >> 1)
        return ("v" if u & 1 else "k"), g, g & (KV_SLOTS - 1)

    phases = [(0, 8, pair_phase("bwq", "bwuk")),
              (8, 8, pair_phase("awq", "bwuv")),
              (16, 16, c_phase),
              (32, 64, kv_phase),
              (96, 8, pair_phase("bwo", "awo"))]

    def phase_of(j):
        for n, (j0, cnt, _) in enumerate(phases):
            if j0 <= j < j0 + cnt:
                return n
        return None

    def copies(ph, j, t, high):
        j0, _, unit = phases[ph]
        name, si, di = unit(j - j0, (t + 2) % 4 if high else t % 4)
        rect, pieces = arrays[name]
        sem = hi_sems.at[j & 3] if high else lo_sems.at[(j & 3) * 16 + t]
        return [pltpu.make_async_copy(*rect(si, di, run), sem)
                for run in pieces[1 if high else 0][t // 4]]

    def start_tick(ph, j, t):
        for cp in copies(ph, j, t, True):
            cp.start(priority=0)
        for cp in copies(ph, j, t, False):
            cp.start(priority=1)

    def wait_tick(ph, j, t):
        if t == 0:
            for tt in range(TICKS):
                for cp in copies(ph, j, tt, True):
                    cp.wait()
        for cp in copies(ph, j, t, False):
            cp.wait()

    def segment(j0, j1, jobs):
        sph = phase_of(j0)
        assert all(phase_of(j) == sph for j in range(j0, j1))
        wphs = sorted({phase_of(j - LAG) for j in range(j0, j1)})

        def iteration(j):
            for t in range(TICKS):
                if len(wphs) == 1:
                    wait_tick(wphs[0], j - LAG, t)
                else:
                    edge = phases[wphs[1]][0] + LAG
                    pl.when(j < edge)(lambda: wait_tick(wphs[0], j - LAG, t))
                    pl.when(j >= edge)(lambda: wait_tick(wphs[1], j - LAG, t))
                if sph is not None:
                    start_tick(sph, j, t)
                if t in jobs:
                    jobs[t](j)

        if j1 - j0 == 1:
            iteration(j0)
        else:
            def body(j, carry):
                iteration(j)
                return carry
            lax.fori_loop(j0, j1, body, 0)

    def repack_job(index):
        def job(j):
            mat, ch = index(j)
            w = w_v[mat, pl.ds(_aligned(ch * 4096, 4096), 4096), :]
            w32_s[mat, ch, pl.ds(0, 2048), :] = pltpu.bitcast(w, U32)
        return job

    def heads(mat, ch, q):
        for hp in range(4 * q, 4 * q + 4):
            lo, hi = _split_pair(w32_s[mat, ch, pl.ds(hp, 128, stride=16), :])
            yield 2 * hp, lo
            yield 2 * hp + 1, hi

    def wq_job(j0, q):
        def job(j):
            x = x8_s[1, j - j0]
            for h, w in heads(0, j - j0, q):
                qb_s[h] += jnp.dot(x, w, preferred_element_type=F32)
        return job

    def wuk_job(j0, q):
        def job(j):
            for h, w in heads(1, j - j0, q):
                qabs_s[pl.ds(8 * h, 8), :] = lax.dot_general(
                    qb_s[h].astype(BF), w, _NT, preferred_element_type=F32)
            if q == 3:
                for b in range(NB):
                    qabs_b[b, j - j0] = qabs_s[pl.ds(b, NH, stride=8), :].astype(BF)
        return job

    def bqk_job(index):
        def job(j):
            n = index(j)
            b = n & 3
            i = c_unit(b, n >> 2)
            q = jnp.concatenate([qabs_b[b, ch] for ch in range(4)], axis=1)
            s = lax.dot_general(q, c_v[i], _NT, preferred_element_type=F32)
            s_s[i] = s
            m_s[b] = jnp.maximum(m_s[b], jnp.maximum(s[:, :128], s[:, 128:]))
        return job

    def bmax_job():
        for b in range(NB):
            m_s[b] = jnp.broadcast_to(jnp.max(m_s[b], axis=-1, keepdims=True), (NH, 128))

    def bpv_job(index):
        def job(j):
            i = index(j)
            b = i >> 4
            m = m_s[b]
            s = s_s[i]
            p0 = jnp.exp((s[:, :128] - m) * SCALE)
            p1 = jnp.exp((s[:, 128:] - m) * SCALE)
            l_s[b] += p0 + p1
            p = jnp.concatenate([p0, p1], axis=1).astype(BF)
            acc_s[b] += jnp.dot(p, c_v[i], preferred_element_type=F32)
        return job

    def bnorm_job():
        for b in range(NB):
            ctxc = acc_s[b] * (1.0 / jnp.sum(l_s[b], axis=-1, keepdims=True))
            for ch in range(4):
                cx_s[ch, pl.ds(b * NH, NH), :] = ctxc[:, ch * 128:(ch + 1) * 128]

    def wuv_job(j0, q):
        def job(j):
            for h, w in heads(2, j - j0, q):
                lhs = cx_s[j - j0, pl.ds(h, 8, stride=NH), :].astype(BF)
                ctx_s[h] += jnp.dot(lhs, w, preferred_element_type=F32)
        return job

    def awq_job(j0, q):
        def job(j):
            half = j - j0
            cols = pl.ds(_aligned(half * 2048, 2048), 2048)
            qa_s[half] += jnp.dot(x8_s[0, q], awq_v[pl.ds(q * 128, 128), cols],
                                  preferred_element_type=F32)
            if q == 3:
                for hh in range(16):
                    qa_b[half * 16 + hh] = qa_s[half, :, hh * 128:(hh + 1) * 128].astype(BF)
        return job

    A0 = 35
    row = lax.broadcasted_iota(jnp.int32, (8, DH), 0)

    def lanes(x):
        return [x[:, c * 128:(c + 1) * 128] for c in range(WIN // 128)]

    def a_scores_job(e, scores=True):
        def job(j):
            if scores:
                g = 2 * (j - A0) + e
                s = lax.dot_general(qa_b[g & (NH - 1)], kbuf[g & (KV_SLOTS - 1)], _NT,
                                    preferred_element_type=F32)
                sa_s[e] = s
                ma_s[e] = _tree(jnp.maximum, lanes(s))
            m = jnp.max(ma_s[1 - e], axis=-1, keepdims=True)
            p = jnp.exp((sa_s[1 - e] - m) * SCALE)
            p_s[1 - e] = p.astype(BF)
            la_s[1 - e] = _tree(jnp.add, lanes(p))
        return job

    def a_values_job(e):
        def job(j):
            g = 2 * (j - A0) + e - 2
            o = jnp.dot(p_s[e], vbuf[g & (KV_SLOTS - 1)], preferred_element_type=F32)
            inv = 1.0 / jnp.sum(la_s[e], axis=-1, keepdims=True)
            h = g & (NH - 1)
            o_s[h] = jnp.where(row == (g >> 5), o * inv, o_s[h])
        return job

    def proj(side, i, halves):
        w_ref, src = ((awo_v, o_s), (bwo_v, ctx_s))[side]
        return sum(jnp.dot(src[2 * i + hf].astype(BF), w_ref[i, pl.ds(hf * 128, 128), :],
                           preferred_element_type=F32) for hf in halves)

    def proj_pair(side, it, halves=(0, 1)):
        return proj(side, mat_unit(it, 0), halves) + proj(side, mat_unit(it, 1), halves)

    def proj_job(side):
        def job(j):
            out_s[side] += proj_pair(side, j - 99)
        return job

    def half_job(side, hf):
        def job(j):
            out_s[side] += proj_pair(side, 7, (hf,))
        return job

    def four(mk):
        return {3 * q + 2: mk(q) for q in range(4)}

    def with_a(x0=None, x1=None):
        if x0 is None:
            return {0: a_values_job(0), 3: a_scores_job(0), 6: a_values_job(1), 9: a_scores_job(1)}
        return {0: a_values_job(0), 2: a_scores_job(0), 4: x0,
                6: a_values_job(1), 8: a_scores_job(1), 10: x1}

    x_copies = [pltpu.make_async_copy(src, x_v.at[n], x_sems.at[n])
                for n, src in enumerate((ax_hbm, bx_hbm))]

    def x_job(j):
        for cp in x_copies:
            cp.wait()
        for n in range(2):
            x8 = jnp.concatenate([x_v[n].astype(F32), jnp.zeros((8 - NB, DM), F32)], axis=0)
            for ch in range(4):
                x8_s[n, ch] = x8[:, ch * 128:(ch + 1) * 128].astype(BF)
        la_s[...] = jnp.ones_like(la_s)
        m_s[...] = jnp.full(m_s.shape, -jnp.inf, F32)

    def zero_job(*refs):
        def job(j):
            for r in refs:
                r[...] = jnp.zeros(r.shape, r.dtype)
        return job

    for j in range(LAG):
        for t in range(TICKS):
            start_tick(0, j, t)
    for cp in x_copies:
        cp.start()

    segment(2, 7, {})
    segment(7, 8, {1: x_job,
                   3: zero_job(qb_s, qabs_s, qa_s, l_s, sa_s, ma_s, p_s, out_s),
                   5: zero_job(acc_s, ctx_s, o_s, w32_s.at[:, :, pl.ds(2048, 16), :]),
                   7: zero_job(cx_s),
                   9: zero_job(vbuf.at[KV_SLOTS - 2]),
                   11: zero_job(vbuf.at[KV_SLOTS - 1])})
    segment(8, 10, {})
    segment(10, 12, four(lambda q: repack_job(lambda j: (j - 10, q))))
    segment(12, 16, four(lambda q: wq_job(12, q)))
    segment(16, 20, four(lambda q: wuk_job(16, q)))
    segment(20, 22, four(lambda q: awq_job(20, q)))
    segment(22, 32, four(lambda q: bqk_job(lambda j: 4 * (j - 22) + q)))
    segment(32, 35, four(lambda q: bqk_job(lambda j: 4 * (j - 22) + q)))
    segment(35, 41, with_a(bqk_job(lambda j: 52 + 2 * (j - 35)), bqk_job(lambda j: 53 + 2 * (j - 35))))
    bmax_job()
    segment(41, 73, with_a(bpv_job(lambda j: 2 * (j - 41)), bpv_job(lambda j: 2 * (j - 41) + 1)))
    bnorm_job()
    segment(73, 75, with_a(repack_job(lambda j: (2, 2 * (j - 73))),
                           repack_job(lambda j: (2, 2 * (j - 73) + 1))))
    segment(75, 79, with_a(wuv_job(75, 0), wuv_job(75, 1)))
    segment(79, 83, with_a(wuv_job(79, 2), wuv_job(79, 3)))
    segment(83, 96, with_a())
    segment(96, 99, with_a())
    segment(99, 100, {0: a_values_job(0), 2: a_scores_job(0, scores=False), 4: a_values_job(1),
                      7: proj_job(1), 10: proj_job(0)})
    segment(100, 104, {3: proj_job(1), 8: proj_job(0)})
    segment(104, 105, {3: proj_job(1), 8: proj_job(0)})
    segment(105, 106, {0: proj_job(1), 2: proj_job(0), 5: half_job(1, 0), 7: half_job(0, 0),
                       9: half_job(1, 1)})
    res = jnp.concatenate([out_s[0] + proj_pair(0, 7, (1,)), out_s[1]], axis=1)
    out_ref[...] = res[:NB, :].astype(out_ref.dtype)


@jax.jit
def pallas_concat_heads__sliding_block_cached__compressed_kv_cla__decode_kernel(
    A_x: jax.Array,
    A_k_cache: jax.Array,
    A_v_cache: jax.Array,
    A_wq: jax.Array,
    A_wo: jax.Array,
    B_x: jax.Array,
    B_c_kv: jax.Array,
    B_w_q: jax.Array,
    B_w_uk: jax.Array,
    B_w_uv: jax.Array,
    B_w_o: jax.Array,
):
    vm = pltpu.VMEM
    scratch = [
        vm((2, NB, DM), BF),
        vm((KV_SLOTS, WIN, DH), BF),
        vm((KV_SLOTS, WIN, DH), BF),
        vm((DM, NH * DH), BF),
        vm((16, 256, DM), BF),
        vm((64, 256, DM), BF),
        vm((3, DM * NH, DH), BF),
        vm((3, 4, 2048 + 16, DH), U32),
        vm((16, 256, DM), BF),
        vm((2, 4, 8, 128), BF),
        vm((NH, 8, DH), F32),
        vm((NH * 8 + 8, 128), F32),
        vm((NB, 4, NH, 128), BF),
        vm((64, NH, 256), F32),
        vm((NB, NH, 128), F32),
        vm((NB, NH, 128), F32),
        vm((NB, NH, DM), F32),
        vm((4, 9 * NH, 128), F32),
        vm((NH, 8, DH), F32),
        vm((2, 8, 2048), F32),
        vm((NH, 8, DH), BF),
        vm((2, 8, WIN), F32),
        vm((2, 8, DH), F32),
        vm((2, 8, WIN), BF),
        vm((2, 8, DH), F32),
        vm((NH, 8, DH), F32),
        vm((2, 8, DM), F32),
        pltpu.SemaphoreType.DMA((64,)),
        pltpu.SemaphoreType.DMA((4,)),
        pltpu.SemaphoreType.DMA((2,)),
    ]
    out = pl.pallas_call(
        _kernel,
        out_shape=jax.ShapeDtypeStruct((NB, 2 * DM), BF),
        in_specs=[pl.BlockSpec(memory_space=pl.ANY)] * 11,
        out_specs=pl.BlockSpec(memory_space=pltpu.VMEM),
        scratch_shapes=scratch,
        compiler_params=pltpu.CompilerParams(
            vmem_limit_bytes=80 * 1024 * 1024,
            disable_bounds_checks=True,
            disable_semaphore_checks=True,
        ),
    )(
        A_x.reshape(NB, DM),
        A_k_cache.reshape(NB * NH, SK, DH),
        A_v_cache.reshape(NB * NH, SK, DH),
        A_wq,
        A_wo.reshape(16, 256, DM),
        B_x.reshape(NB, DM),
        B_c_kv.reshape(64, 256, DM),
        B_w_q.reshape(DM * NH, DH),
        B_w_uk.reshape(DM * NH, DH),
        B_w_uv.reshape(DM * NH, DH),
        B_w_o.reshape(16, 256, DM),
    )
    return out.reshape(NB, 1, 2 * DM)
```

```python
import jax
import jax.numpy as jnp
from jax import lax
from jax.experimental import pallas as pl
from jax.experimental.pallas import tpu as pltpu

BF = jnp.bfloat16
F32 = jnp.float32
U32 = jnp.uint32

NB = 4
NH = 32
DH = 128
SK = 4096
WIN = 1024
DM = 512
SCALE = float(DH) ** -0.5

KV_SLOTS = 16
LAG = 2
TICKS = 12
NIT = 104

CUT_A = 15
CUT_B = 17

_NT = (((1,), (1,)), ((), ()))


def _split_pair(w):
    lo = pltpu.bitcast(w << 16, F32).astype(BF)
    hi = pltpu.bitcast(w & U32(0xFFFF0000), F32).astype(BF)
    return lo, hi


def _tree(op, parts):
    while len(parts) > 1:
        parts = [op(parts[2 * c], parts[2 * c + 1]) for c in range(len(parts) // 2)]
    return parts[0]


def _unit_pieces(cut):
    mid = (cut + 96 + 128) // 2
    lo = [(cut + 32 * p, 32) for p in range(3)]
    hi = [(0, cut), (cut + 96, mid - cut - 96), (mid, 128 - mid)]
    return lo, hi


def _tile_major(x, units):
    r, c = x.shape
    return x.reshape(r // 8, 8, c // 128, 128).transpose(0, 2, 1, 3).reshape(units, 128, 8, 128)


def _untile(t, ncol, c0=0, c1=None):
    t = t.reshape(t.shape[0] // ncol, ncol, 8, 128)
    cols = range(c0, ncol if c1 is None else c1)
    return jnp.concatenate([t[:, c].reshape(-1, 128) for c in cols], axis=1)


def _aligned(x, m):
    return x if isinstance(x, int) else pl.multiple_of(x, m)


def _kernel(ax_hbm, k_hbm, v_hbm, awq_hbm, awo_hbm,
            bx_hbm, c_hbm, bwq_hbm, bwuk_hbm, bwuv_hbm, bwo_hbm,
            out_ref,
            x_v, kbuf, vbuf, awq_v, awo_v, c_v, w_v, w32_s, bwo_v,
            x8_s, qb_s, qabs_s, qabs_b, s_s, m_s, l_s, acc_s, cx_s, ctx_s,
            qa_s, qa_b, sa_s, ma_s, p_s, la_s, o_s, out_s,
            lo_sems, hi_sems, x_sems):

    def tiled(hbm, vmem, cut):
        def piece(si, di, t0, n):
            return hbm.at[si, pl.ds(t0, n)], vmem.at[di, pl.ds(t0, n)]
        return piece, _unit_pieces(cut)

    def window(hbm, vmem):
        def piece(si, di, t0, n):
            return (hbm.at[si, pl.ds(SK - WIN + 8 * t0, 8 * n), :],
                    vmem.at[di, pl.ds(8 * t0, 8 * n), :])
        return piece, _unit_pieces(CUT_A)

    def rows(hbm, vmem):
        def piece(si, di, t0, n):
            rs = pl.ds(_aligned(si * 1024 + 8 * t0, 8), 8 * n)
            return hbm.at[rs, :], vmem.at[rs, :]
        return piece, _unit_pieces(CUT_B)

    arrays = dict(
        bwq=rows(bwq_hbm, w_v.at[0]),
        bwuk=rows(bwuk_hbm, w_v.at[1]),
        bwuv=rows(bwuv_hbm, w_v.at[2]),
        awq=tiled(awq_hbm, awq_v, CUT_A),
        c=tiled(c_hbm, c_v, CUT_B),
        bwo=tiled(bwo_hbm, bwo_v, CUT_B),
        awo=tiled(awo_hbm, awo_v, CUT_A),
        k=window(k_hbm, kbuf),
        v=window(v_hbm, vbuf),
    )

    def mat_unit(it, u):
        return 2 * ((it & 3) + 4 * (u & 1)) + (it >> 2)

    def c_unit(b, it):
        return 16 * b + 2 * (it & 7) + (it >> 3)

    def pair_phase(a, b):
        def unit(it, u):
            i = mat_unit(it, u)
            return (a if u < 2 else b), i, i
        return unit

    def c_phase(it, u):
        i = c_unit(u, it)
        return "c", i, i

    def kv_phase(it, u):
        g = 2 * it + (u >> 1)
        return ("v" if u & 1 else "k"), g, g & (KV_SLOTS - 1)

    phases = [(0, 8, pair_phase("bwq", "bwuk")),
              (8, 8, pair_phase("awq", "bwuv")),
              (16, 16, c_phase),
              (32, 64, kv_phase),
              (96, 8, pair_phase("bwo", "awo"))]

    def phase_of(j):
        for n, (j0, cnt, _) in enumerate(phases):
            if j0 <= j < j0 + cnt:
                return n
        return None

    def copy(ph, j, t, high):
        j0, _, unit = phases[ph]
        name, si, di = unit(j - j0, (t + 2) % 4 if high else t % 4)
        piece, ranges = arrays[name]
        sem = hi_sems.at[j & 3] if high else lo_sems.at[(j & 3) * 16 + t]
        return pltpu.make_async_copy(*piece(si, di, *ranges[high][t // 4]), sem)

    def start_tick(ph, j, t):
        copy(ph, j, t, True).start(priority=0)
        copy(ph, j, t, False).start(priority=1)

    def wait_tick(ph, j, t):
        if t == 0:
            for tt in range(TICKS):
                copy(ph, j, tt, True).wait()
        copy(ph, j, t, False).wait()

    def segment(j0, j1, jobs):
        sph = phase_of(j0)
        assert all(phase_of(j) == sph for j in range(j0, j1))
        wphs = sorted({phase_of(j - LAG) for j in range(j0, j1)})

        def iteration(j):
            for t in range(TICKS):
                if len(wphs) == 1:
                    wait_tick(wphs[0], j - LAG, t)
                else:
                    edge = phases[wphs[1]][0] + LAG
                    pl.when(j < edge)(lambda: wait_tick(wphs[0], j - LAG, t))
                    pl.when(j >= edge)(lambda: wait_tick(wphs[1], j - LAG, t))
                if sph is not None:
                    start_tick(sph, j, t)
                if t in jobs:
                    jobs[t](j)

        if j1 - j0 == 1:
            iteration(j0)
        else:
            def body(j, carry):
                iteration(j)
                return carry
            lax.fori_loop(j0, j1, body, 0)

    def repack_job(index):
        def job(j):
            mat, ch = index(j)
            w = w_v[mat, pl.ds(_aligned(ch * 4096, 4096), 4096), :]
            w32_s[mat, ch, pl.ds(0, 2048), :] = pltpu.bitcast(w, U32)
        return job

    def heads(mat, ch, q):
        for hp in range(4 * q, 4 * q + 4):
            lo, hi = _split_pair(w32_s[mat, ch, pl.ds(hp, 128, stride=16), :])
            yield 2 * hp, lo
            yield 2 * hp + 1, hi

    def wq_job(j0, q):
        def job(j):
            x = x8_s[1, j - j0]
            for h, w in heads(0, j - j0, q):
                qb_s[h] += jnp.dot(x, w, preferred_element_type=F32)
        return job

    def wuk_job(j0, q):
        def job(j):
            for h, w in heads(1, j - j0, q):
                qabs_s[pl.ds(8 * h, 8), :] = lax.dot_general(
                    qb_s[h].astype(BF), w, _NT, preferred_element_type=F32)
            if q == 3:
                for b in range(NB):
                    qabs_b[b, j - j0] = qabs_s[pl.ds(b, NH, stride=8), :].astype(BF)
        return job

    def bqk_job(index):
        def job(j):
            n = index(j)
            b = n & 3
            i = c_unit(b, n >> 2)
            q = jnp.concatenate([qabs_b[b, ch] for ch in range(4)], axis=1)
            s = lax.dot_general(q, _untile(c_v[i], 4), _NT, preferred_element_type=F32)
            s_s[i] = s
            m_s[b] = jnp.maximum(m_s[b], jnp.maximum(s[:, :128], s[:, 128:]))
        return job

    def bmax_job():
        for b in range(NB):
            m_s[b] = jnp.broadcast_to(jnp.max(m_s[b], axis=-1, keepdims=True), (NH, 128))

    def bpv_job(index):
        def job(j):
            i = index(j)
            b = i >> 4
            m = m_s[b]
            s = s_s[i]
            p0 = jnp.exp((s[:, :128] - m) * SCALE)
            p1 = jnp.exp((s[:, 128:] - m) * SCALE)
            l_s[b] += p0 + p1
            p = jnp.concatenate([p0, p1], axis=1).astype(BF)
            acc_s[b] += jnp.dot(p, _untile(c_v[i], 4), preferred_element_type=F32)
        return job

    def bnorm_job():
        for b in range(NB):
            ctxc = acc_s[b] * (1.0 / jnp.sum(l_s[b], axis=-1, keepdims=True))
            for ch in range(4):
                cx_s[ch, pl.ds(b * NH, NH), :] = ctxc[:, ch * 128:(ch + 1) * 128]

    def wuv_job(j0, q):
        def job(j):
            for h, w in heads(2, j - j0, q):
                lhs = cx_s[j - j0, pl.ds(h, 8, stride=NH), :].astype(BF)
                ctx_s[h] += jnp.dot(lhs, w, preferred_element_type=F32)
        return job

    def awq_job(j0, n):
        def job(j):
            ch = 2 * (j - j0) + (n >> 1)
            half = n & 1
            w = awq_v[pl.ds(4 * ch, 4)].reshape(512, 8, 128)
            qa_s[half] += jnp.dot(x8_s[0, ch], _untile(w, 32, 16 * half, 16 * half + 16),
                                  preferred_element_type=F32)
        return job

    def aq_cast_job():
        for h in range(NH):
            qa_b[h] = qa_s[h // 16, :, (h % 16) * 128:(h % 16 + 1) * 128].astype(BF)

    A0 = 35
    row = lax.broadcasted_iota(jnp.int32, (8, DH), 0)

    def lanes(x):
        return [x[:, c * 128:(c + 1) * 128] for c in range(WIN // 128)]

    def a_scores_job(e, scores=True):
        def job(j):
            if scores:
                g = 2 * (j - A0) + e
                s = lax.dot_general(qa_b[g & (NH - 1)], kbuf[g & (KV_SLOTS - 1)], _NT,
                                    preferred_element_type=F32)
                sa_s[e] = s
                ma_s[e] = _tree(jnp.maximum, lanes(s))
            m = jnp.max(ma_s[1 - e], axis=-1, keepdims=True)
            p = jnp.exp((sa_s[1 - e] - m) * SCALE)
            p_s[1 - e] = p.astype(BF)
            la_s[1 - e] = _tree(jnp.add, lanes(p))
        return job

    def a_values_job(e):
        def job(j):
            g = 2 * (j - A0) + e - 2
            o = jnp.dot(p_s[e], vbuf[g & (KV_SLOTS - 1)], preferred_element_type=F32)
            inv = 1.0 / jnp.sum(la_s[e], axis=-1, keepdims=True)
            h = g & (NH - 1)
            o_s[h] = jnp.where(row == (g >> 5), o * inv, o_s[h])
        return job

    def proj(side, i, halves):
        w_ref, src = ((awo_v, o_s), (bwo_v, ctx_s))[side]
        return sum(jnp.dot(src[2 * i + hf].astype(BF), _untile(w_ref[i, pl.ds(hf * 64, 64)], 4),
                           preferred_element_type=F32) for hf in halves)

    def proj_pair(side, it, halves=(0, 1)):
        return proj(side, mat_unit(it, 0), halves) + proj(side, mat_unit(it, 1), halves)

    def proj_job(side):
        def job(j):
            out_s[side] += proj_pair(side, j - 99)
        return job

    def half_job(side, hf):
        def job(j):
            out_s[side] += proj_pair(side, 7, (hf,))
        return job

    def four(mk):
        return {3 * q + 2: mk(q) for q in range(4)}

    def with_a(x0=None, x1=None):
        if x0 is None:
            return {0: a_values_job(0), 3: a_scores_job(0), 6: a_values_job(1), 9: a_scores_job(1)}
        return {0: a_values_job(0), 2: a_scores_job(0), 4: x0,
                6: a_values_job(1), 8: a_scores_job(1), 10: x1}

    x_copies = [pltpu.make_async_copy(src, x_v.at[n], x_sems.at[n])
                for n, src in enumerate((ax_hbm, bx_hbm))]

    def x_job(j):
        for cp in x_copies:
            cp.wait()
        for n in range(2):
            x8 = jnp.concatenate([x_v[n].astype(F32), jnp.zeros((8 - NB, DM), F32)], axis=0)
            for ch in range(4):
                x8_s[n, ch] = x8[:, ch * 128:(ch + 1) * 128].astype(BF)
        la_s[...] = jnp.ones_like(la_s)
        m_s[...] = jnp.full(m_s.shape, -jnp.inf, F32)

    def zero_job(*refs):
        def job(j):
            for r in refs:
                r[...] = jnp.zeros(r.shape, r.dtype)
        return job

    for j in range(LAG):
        for t in range(TICKS):
            start_tick(0, j, t)
    for cp in x_copies:
        cp.start()

    segment(2, 7, {})
    segment(7, 8, {1: x_job,
                   3: zero_job(qb_s, qabs_s, qa_s, l_s, sa_s, ma_s, p_s, out_s),
                   5: zero_job(acc_s, ctx_s, o_s, w32_s.at[:, :, pl.ds(2048, 16), :]),
                   7: zero_job(cx_s),
                   9: zero_job(vbuf.at[KV_SLOTS - 2]),
                   11: zero_job(vbuf.at[KV_SLOTS - 1])})
    segment(8, 10, {})
    segment(10, 12, four(lambda q: repack_job(lambda j: (j - 10, q))))
    segment(12, 16, four(lambda q: wq_job(12, q)))
    segment(16, 20, four(lambda q: wuk_job(16, q)))
    segment(20, 22, four(lambda q: awq_job(20, q)))
    aq_cast_job()
    segment(22, 32, four(lambda q: bqk_job(lambda j: 4 * (j - 22) + q)))
    segment(32, 35, four(lambda q: bqk_job(lambda j: 4 * (j - 22) + q)))
    segment(35, 41, with_a(bqk_job(lambda j: 52 + 2 * (j - 35)), bqk_job(lambda j: 53 + 2 * (j - 35))))
    bmax_job()
    segment(41, 73, with_a(bpv_job(lambda j: 2 * (j - 41)), bpv_job(lambda j: 2 * (j - 41) + 1)))
    bnorm_job()
    segment(73, 75, with_a(repack_job(lambda j: (2, 2 * (j - 73))),
                           repack_job(lambda j: (2, 2 * (j - 73) + 1))))
    segment(75, 79, with_a(wuv_job(75, 0), wuv_job(75, 1)))
    segment(79, 83, with_a(wuv_job(79, 2), wuv_job(79, 3)))
    segment(83, 96, with_a())
    segment(96, 99, with_a())
    segment(99, 100, {0: a_values_job(0), 2: a_scores_job(0, scores=False), 4: a_values_job(1),
                      7: proj_job(1), 10: proj_job(0)})
    segment(100, 104, {3: proj_job(1), 8: proj_job(0)})
    segment(104, 105, {3: proj_job(1), 8: proj_job(0)})
    segment(105, 106, {0: proj_job(1), 2: proj_job(0), 5: half_job(1, 0), 7: half_job(0, 0),
                       9: half_job(1, 1)})
    res = jnp.concatenate([out_s[0] + proj_pair(0, 7, (1,)), out_s[1]], axis=1)
    out_ref[...] = res[:NB, :].astype(out_ref.dtype)


@jax.jit
def pallas_concat_heads__sliding_block_cached__compressed_kv_cla__decode_kernel(
    A_x: jax.Array,
    A_k_cache: jax.Array,
    A_v_cache: jax.Array,
    A_wq: jax.Array,
    A_wo: jax.Array,
    B_x: jax.Array,
    B_c_kv: jax.Array,
    B_w_q: jax.Array,
    B_w_uk: jax.Array,
    B_w_uv: jax.Array,
    B_w_o: jax.Array,
):
    vm = pltpu.VMEM
    scratch = [
        vm((2, NB, DM), BF),
        vm((KV_SLOTS, WIN, DH), BF),
        vm((KV_SLOTS, WIN, DH), BF),
        vm((16, 128, 8, 128), BF),
        vm((16, 128, 8, 128), BF),
        vm((64, 128, 8, 128), BF),
        vm((3, DM * NH, DH), BF),
        vm((3, 4, 2048 + 16, DH), U32),
        vm((16, 128, 8, 128), BF),
        vm((2, 4, 8, 128), BF),
        vm((NH, 8, DH), F32),
        vm((NH * 8 + 8, 128), F32),
        vm((NB, 4, NH, 128), BF),
        vm((64, NH, 256), F32),
        vm((NB, NH, 128), F32),
        vm((NB, NH, 128), F32),
        vm((NB, NH, DM), F32),
        vm((4, 9 * NH, 128), F32),
        vm((NH, 8, DH), F32),
        vm((2, 8, 2048), F32),
        vm((NH, 8, DH), BF),
        vm((2, 8, WIN), F32),
        vm((2, 8, DH), F32),
        vm((2, 8, WIN), BF),
        vm((2, 8, DH), F32),
        vm((NH, 8, DH), F32),
        vm((2, 8, DM), F32),
        pltpu.SemaphoreType.DMA((64,)),
        pltpu.SemaphoreType.DMA((4,)),
        pltpu.SemaphoreType.DMA((2,)),
    ]
    out = pl.pallas_call(
        _kernel,
        out_shape=jax.ShapeDtypeStruct((NB, 2 * DM), BF),
        in_specs=[pl.BlockSpec(memory_space=pl.ANY)] * 11,
        out_specs=pl.BlockSpec(memory_space=pltpu.VMEM),
        scratch_shapes=scratch,
        compiler_params=pltpu.CompilerParams(
            vmem_limit_bytes=80 * 1024 * 1024,
            disable_bounds_checks=True,
            disable_semaphore_checks=True,
        ),
    )(
        A_x.reshape(NB, DM),
        A_k_cache.reshape(NB * NH, SK, DH),
        A_v_cache.reshape(NB * NH, SK, DH),
        _tile_major(A_wq, 16),
        _tile_major(A_wo, 16),
        B_x.reshape(NB, DM),
        _tile_major(B_c_kv.reshape(NB * SK, DM), 64),
        B_w_q.reshape(DM * NH, DH),
        B_w_uk.reshape(DM * NH, DH),
        B_w_uv.reshape(DM * NH, DH),
        _tile_major(B_w_o.reshape(NH * DH, DM), 16),
    )
    return out.reshape(NB, 1, 2 * DM)
```

```python
import jax
import jax.numpy as jnp
from jax import lax
from jax.experimental import pallas as pl
from jax.experimental.pallas import tpu as pltpu

BF = jnp.bfloat16
F32 = jnp.float32
U32 = jnp.uint32

NB = 4
NH = 32
DH = 128
SK = 4096
WIN = 1024
DM = 512
SCALE = float(DH) ** -0.5

KV_SLOTS = 16
LAG = 2
TICKS = 12

CUT_A = 15
CUT_B = 17

_NT = (((1,), (1,)), ((), ()))


def _split_pair(w):
    lo = pltpu.bitcast(w << 16, F32).astype(BF)
    hi = pltpu.bitcast(w & U32(0xFFFF0000), F32).astype(BF)
    return lo, hi


def _tree(op, parts):
    while len(parts) > 1:
        parts = [op(parts[2 * c], parts[2 * c + 1]) for c in range(len(parts) // 2)]
    return parts[0]


def _unit_pieces(cut):
    mid = (cut + 96 + 128) // 2
    lo = [(cut + 32 * p, 32) for p in range(3)]
    hi = [(0, cut), (cut + 96, mid - cut - 96), (mid, 128 - mid)]
    return lo, hi


def _tile_major(x, units):
    r, c = x.shape
    return x.reshape(r // 8, 8, c // 128, 128).transpose(0, 2, 1, 3).reshape(units, 128, 8, 128)


def _untile(t, ncol, c0=0, c1=None):
    t = t.reshape(t.shape[0] // ncol, ncol, 8, 128)
    cols = range(c0, ncol if c1 is None else c1)
    return jnp.concatenate([t[:, c].reshape(-1, 128) for c in cols], axis=1)


def _aligned(x, m):
    return x if isinstance(x, int) else pl.multiple_of(x, m)


def _kernel(ax_hbm, k_hbm, v_hbm, awq_hbm, awo_hbm,
            bx_hbm, c_hbm, bwq_hbm, bwuk_hbm, bwuv_hbm, bwo_hbm,
            out_ref,
            x_v, kbuf, vbuf, awq_v, awo_v, c_v, w_v, w32_s, bwo_v,
            x8_s, qb_s, qabs_s, qabs_b, s_s, m_s, l_s, acc_s, cx_s, ctx_s,
            qa_s, qa_b, sa_s, ma_s, p_s, la_s, o_s, out_s,
            lo_sems, hi_sems, x_sems):

    def tiled(hbm, vmem, cut):
        def piece(si, di, t0, n):
            return hbm.at[si, pl.ds(t0, n)], vmem.at[di, pl.ds(t0, n)]
        return piece, _unit_pieces(cut)

    def window(hbm, vmem):
        def piece(si, di, t0, n):
            return (hbm.at[si, pl.ds(SK - WIN + 8 * t0, 8 * n), :],
                    vmem.at[di, pl.ds(8 * t0, 8 * n), :])
        return piece, _unit_pieces(CUT_A)

    def rows(hbm, vmem):
        def piece(si, di, t0, n):
            rs = pl.ds(_aligned(si * 1024 + 8 * t0, 8), 8 * n)
            return hbm.at[rs, :], vmem.at[rs, :]
        return piece, _unit_pieces(CUT_B)

    arrays = dict(
        bwq=rows(bwq_hbm, w_v.at[0]),
        bwuk=rows(bwuk_hbm, w_v.at[1]),
        bwuv=rows(bwuv_hbm, w_v.at[2]),
        awq=tiled(awq_hbm, awq_v, CUT_A),
        c=tiled(c_hbm, c_v, CUT_B),
        bwo=tiled(bwo_hbm, bwo_v, CUT_B),
        awo=tiled(awo_hbm, awo_v, CUT_A),
        k=window(k_hbm, kbuf),
        v=window(v_hbm, vbuf),
    )

    def mat_unit(it, u):
        return 2 * (3 - (it & 3) + 4 * (u & 1)) + (it >> 2)

    def c_unit(b, it):
        return 16 * b + 2 * (7 - (it & 7)) + (it >> 3)

    def pair_phase(a, b):
        def unit(it, u):
            i = mat_unit(it, u)
            return (a if u < 2 else b), i, i
        return unit

    def c_phase(it, u):
        i = c_unit(u, it)
        return "c", i, i

    def kv_phase(it, u):
        g = 2 * it + (u >> 1)
        return ("v" if u & 1 else "k"), g, g & (KV_SLOTS - 1)

    phases = [(0, 8, pair_phase("bwq", "bwuk")),
              (8, 8, pair_phase("awq", "bwuv")),
              (16, 16, c_phase),
              (32, 64, kv_phase),
              (96, 8, pair_phase("bwo", "awo"))]

    def phase_of(j):
        for n, (j0, cnt, _) in enumerate(phases):
            if j0 <= j < j0 + cnt:
                return n
        return None

    def copy(ph, j, t, high):
        j0, _, unit = phases[ph]
        if high:
            q = t % 3
            u = (t // 3 + (2 if q else 0)) % 4
        else:
            q, u = divmod(t, 4)
        name, si, di = unit(j - j0, u)
        piece, ranges = arrays[name]
        sem = hi_sems.at[j & 3] if high else lo_sems.at[(j & 3) * 16 + t]
        return pltpu.make_async_copy(*piece(si, di, *ranges[high][q]), sem)

    def start_tick(ph, j, t):
        copy(ph, j, t, False).start(priority=1)
        copy(ph, j, t, True).start(priority=0)

    def wait_tick(ph, j, t):
        if t == 0:
            for tt in range(TICKS):
                copy(ph, j, tt, True).wait()
        copy(ph, j, t, False).wait()

    def segment(j0, j1, jobs):
        sph = phase_of(j0)
        assert all(phase_of(j) == sph for j in range(j0, j1))
        wphs = sorted({phase_of(j - LAG) for j in range(j0, j1)})

        def iteration(j):
            for t in range(TICKS):
                if len(wphs) == 1:
                    wait_tick(wphs[0], j - LAG, t)
                else:
                    edge = phases[wphs[1]][0] + LAG
                    pl.when(j < edge)(lambda: wait_tick(wphs[0], j - LAG, t))
                    pl.when(j >= edge)(lambda: wait_tick(wphs[1], j - LAG, t))
                if sph is not None:
                    start_tick(sph, j, t)
                if t in jobs:
                    jobs[t](j)

        if j1 - j0 == 1:
            iteration(j0)
        else:
            def body(j, carry):
                iteration(j)
                return carry
            lax.fori_loop(j0, j1, body, 0)

    def repack_job(index):
        def job(j):
            mat, ch = index(j)
            w = w_v[mat, pl.ds(_aligned(ch * 4096, 4096), 4096), :]
            w32_s[mat, ch, pl.ds(0, 2048), :] = pltpu.bitcast(w, U32)
        return job

    def heads(mat, ch, q):
        for hp in range(4 * q, 4 * q + 4):
            lo, hi = _split_pair(w32_s[mat, ch, pl.ds(hp, 128, stride=16), :])
            yield 2 * hp, lo
            yield 2 * hp + 1, hi

    def wq_job(j0, q):
        def job(j):
            x = x8_s[1, j - j0]
            for h, w in heads(0, j - j0, q):
                qb_s[h] += jnp.dot(x, w, preferred_element_type=F32)
        return job

    def wuk_job(j0, q):
        def job(j):
            for h, w in heads(1, j - j0, q):
                qabs_s[pl.ds(8 * h, 8), :] = lax.dot_general(
                    qb_s[h].astype(BF), w, _NT, preferred_element_type=F32)
            if q == 3:
                for b in range(NB):
                    qabs_b[b, j - j0] = qabs_s[pl.ds(b, NH, stride=8), :].astype(BF)
        return job

    def bqk_job(index):
        def job(j):
            n = index(j)
            b = n & 3
            i = c_unit(b, n >> 2)
            q = jnp.concatenate([qabs_b[b, ch] for ch in range(4)], axis=1)
            s = lax.dot_general(q, _untile(c_v[i], 4), _NT, preferred_element_type=F32)
            s_s[i] = s
            m_s[b] = jnp.maximum(m_s[b], jnp.maximum(s[:, :128], s[:, 128:]))
        return job

    def bmax_job():
        for b in range(NB):
            m_s[b] = jnp.broadcast_to(jnp.max(m_s[b], axis=-1, keepdims=True), (NH, 128))

    def bpv_job(index):
        def job(j):
            i = index(j)
            b = i >> 4
            m = m_s[b]
            s = s_s[i]
            p0 = jnp.exp((s[:, :128] - m) * SCALE)
            p1 = jnp.exp((s[:, 128:] - m) * SCALE)
            l_s[b] += p0 + p1
            p = jnp.concatenate([p0, p1], axis=1).astype(BF)
            acc_s[b] += jnp.dot(p, _untile(c_v[i], 4), preferred_element_type=F32)
        return job

    def bnorm_job():
        for b in range(NB):
            ctxc = acc_s[b] * (1.0 / jnp.sum(l_s[b], axis=-1, keepdims=True))
            for ch in range(4):
                cx_s[ch, pl.ds(b * NH, NH), :] = ctxc[:, ch * 128:(ch + 1) * 128]

    def wuv_job(j0, q):
        def job(j):
            for h, w in heads(2, j - j0, q):
                lhs = cx_s[j - j0, pl.ds(h, 8, stride=NH), :].astype(BF)
                ctx_s[h] += jnp.dot(lhs, w, preferred_element_type=F32)
        return job

    def awq_job(j0, n):
        def job(j):
            ch = 2 * (j - j0) + (n >> 1)
            half = n & 1
            w = awq_v[pl.ds(4 * ch, 4)].reshape(512, 8, 128)
            qa_s[half] += jnp.dot(x8_s[0, ch], _untile(w, 32, 16 * half, 16 * half + 16),
                                  preferred_element_type=F32)
        return job

    def aq_cast_job():
        for h in range(NH):
            qa_b[h] = qa_s[h // 16, :, (h % 16) * 128:(h % 16 + 1) * 128].astype(BF)

    A0 = 35
    row = lax.broadcasted_iota(jnp.int32, (8, DH), 0)

    def lanes(x):
        return [x[:, c * 128:(c + 1) * 128] for c in range(WIN // 128)]

    def a_scores_job(e, scores=True):
        def job(j):
            if scores:
                g = 2 * (j - A0) + e
                s = lax.dot_general(qa_b[g & (NH - 1)], kbuf[g & (KV_SLOTS - 1)], _NT,
                                    preferred_element_type=F32)
                sa_s[e] = s
                ma_s[e] = _tree(jnp.maximum, lanes(s))
            m = jnp.max(ma_s[1 - e], axis=-1, keepdims=True)
            p = jnp.exp((sa_s[1 - e] - m) * SCALE)
            p_s[1 - e] = p.astype(BF)
            la_s[1 - e] = _tree(jnp.add, lanes(p))
        return job

    def a_values_job(e):
        def job(j):
            g = 2 * (j - A0) + e - 2
            o = jnp.dot(p_s[e], vbuf[g & (KV_SLOTS - 1)], preferred_element_type=F32)
            inv = 1.0 / jnp.sum(la_s[e], axis=-1, keepdims=True)
            h = g & (NH - 1)
            o_s[h] = jnp.where(row == (g >> 5), o * inv, o_s[h])
        return job

    def proj(side, i, halves):
        w_ref, src = ((awo_v, o_s), (bwo_v, ctx_s))[side]
        return sum(jnp.dot(src[2 * i + hf].astype(BF), _untile(w_ref[i, pl.ds(hf * 64, 64)], 4),
                           preferred_element_type=F32) for hf in halves)

    def proj_pair(side, it, halves=(0, 1)):
        return proj(side, mat_unit(it, 0), halves) + proj(side, mat_unit(it, 1), halves)

    def proj_job(side):
        def job(j):
            out_s[side] += proj_pair(side, j - 99)
        return job

    def half_job(side, hf):
        def job(j):
            out_s[side] += proj_pair(side, 7, (hf,))
        return job

    def four(mk):
        return {3 * q: mk(q) for q in range(4)}

    def with_a(x0=None, x1=None):
        if x0 is None:
            return {0: a_values_job(0), 3: a_scores_job(0), 6: a_values_job(1), 9: a_scores_job(1)}
        return {0: a_values_job(0), 2: a_scores_job(0), 4: x0,
                6: a_values_job(1), 8: a_scores_job(1), 10: x1}

    x_copies = [pltpu.make_async_copy(src, x_v.at[n], x_sems.at[n])
                for n, src in enumerate((ax_hbm, bx_hbm))]

    def x_job(j):
        for cp in x_copies:
            cp.wait()
        for n in range(2):
            x8 = jnp.concatenate([x_v[n].astype(F32), jnp.zeros((8 - NB, DM), F32)], axis=0)
            for ch in range(4):
                x8_s[n, ch] = x8[:, ch * 128:(ch + 1) * 128].astype(BF)
        la_s[...] = jnp.ones_like(la_s)
        m_s[...] = jnp.full(m_s.shape, -jnp.inf, F32)

    def zero_job(*refs):
        def job(j):
            for r in refs:
                r[...] = jnp.zeros(r.shape, r.dtype)
        return job

    for j in range(LAG):
        for t in range(TICKS):
            start_tick(0, j, t)
    for cp in x_copies:
        cp.start()

    segment(2, 7, {})
    segment(7, 8, {1: x_job,
                   3: zero_job(qb_s, qabs_s, qa_s, l_s, sa_s, ma_s, p_s, out_s),
                   5: zero_job(acc_s, ctx_s, o_s, w32_s.at[:, :, pl.ds(2048, 16), :]),
                   7: zero_job(cx_s),
                   9: zero_job(vbuf.at[KV_SLOTS - 2]),
                   11: zero_job(vbuf.at[KV_SLOTS - 1])})
    segment(8, 10, {})
    segment(10, 12, four(lambda q: repack_job(lambda j: (j - 10, q))))
    segment(12, 16, four(lambda q: wq_job(12, q)))
    segment(16, 20, four(lambda q: wuk_job(16, q)))
    segment(20, 22, four(lambda q: awq_job(20, q)))
    aq_cast_job()
    segment(22, 32, four(lambda q: bqk_job(lambda j: 4 * (j - 22) + q)))
    segment(32, 35, four(lambda q: bqk_job(lambda j: 4 * (j - 22) + q)))
    segment(35, 41, with_a(bqk_job(lambda j: 52 + 2 * (j - 35)), bqk_job(lambda j: 53 + 2 * (j - 35))))
    bmax_job()
    segment(41, 73, with_a(bpv_job(lambda j: 2 * (j - 41)), bpv_job(lambda j: 2 * (j - 41) + 1)))
    bnorm_job()
    segment(73, 75, with_a(repack_job(lambda j: (2, 2 * (j - 73))),
                           repack_job(lambda j: (2, 2 * (j - 73) + 1))))
    segment(75, 79, with_a(wuv_job(75, 0), wuv_job(75, 1)))
    segment(79, 83, with_a(wuv_job(79, 2), wuv_job(79, 3)))
    segment(83, 96, with_a())
    segment(96, 99, with_a())
    segment(99, 100, {0: a_values_job(0), 2: a_scores_job(0, scores=False), 4: a_values_job(1),
                      7: proj_job(1), 10: proj_job(0)})
    segment(100, 104, {3: proj_job(1), 8: proj_job(0)})
    segment(104, 105, {3: proj_job(1), 8: proj_job(0)})
    segment(105, 106, {0: proj_job(1), 2: proj_job(0), 5: half_job(1, 0), 7: half_job(0, 0),
                       9: half_job(1, 1)})
    res = jnp.concatenate([out_s[0] + proj_pair(0, 7, (1,)), out_s[1]], axis=1)
    out_ref[...] = res[:NB, :].astype(out_ref.dtype)


@jax.jit
def pallas_concat_heads__sliding_block_cached__compressed_kv_cla__decode_kernel(
    A_x: jax.Array,
    A_k_cache: jax.Array,
    A_v_cache: jax.Array,
    A_wq: jax.Array,
    A_wo: jax.Array,
    B_x: jax.Array,
    B_c_kv: jax.Array,
    B_w_q: jax.Array,
    B_w_uk: jax.Array,
    B_w_uv: jax.Array,
    B_w_o: jax.Array,
):
    vm = pltpu.VMEM
    scratch = [
        vm((2, NB, DM), BF),
        vm((KV_SLOTS, WIN, DH), BF),
        vm((KV_SLOTS, WIN, DH), BF),
        vm((16, 128, 8, 128), BF),
        vm((16, 128, 8, 128), BF),
        vm((64, 128, 8, 128), BF),
        vm((3, DM * NH, DH), BF),
        vm((3, 4, 2048 + 16, DH), U32),
        vm((16, 128, 8, 128), BF),
        vm((2, 4, 8, 128), BF),
        vm((NH, 8, DH), F32),
        vm((NH * 8 + 8, 128), F32),
        vm((NB, 4, NH, 128), BF),
        vm((64, NH, 256), F32),
        vm((NB, NH, 128), F32),
        vm((NB, NH, 128), F32),
        vm((NB, NH, DM), F32),
        vm((4, 9 * NH, 128), F32),
        vm((NH, 8, DH), F32),
        vm((2, 8, 2048), F32),
        vm((NH, 8, DH), BF),
        vm((2, 8, WIN), F32),
        vm((2, 8, DH), F32),
        vm((2, 8, WIN), BF),
        vm((2, 8, DH), F32),
        vm((NH, 8, DH), F32),
        vm((2, 8, DM), F32),
        pltpu.SemaphoreType.DMA((64,)),
        pltpu.SemaphoreType.DMA((4,)),
        pltpu.SemaphoreType.DMA((2,)),
    ]
    out = pl.pallas_call(
        _kernel,
        out_shape=jax.ShapeDtypeStruct((NB, 2 * DM), BF),
        in_specs=[pl.BlockSpec(memory_space=pl.ANY)] * 11,
        out_specs=pl.BlockSpec(memory_space=pltpu.VMEM),
        scratch_shapes=scratch,
        compiler_params=pltpu.CompilerParams(
            vmem_limit_bytes=80 * 1024 * 1024,
            disable_bounds_checks=True,
            disable_semaphore_checks=True,
        ),
    )(
        A_x.reshape(NB, DM),
        A_k_cache.reshape(NB * NH, SK, DH),
        A_v_cache.reshape(NB * NH, SK, DH),
        _tile_major(A_wq, 16),
        _tile_major(A_wo, 16),
        B_x.reshape(NB, DM),
        _tile_major(B_c_kv.reshape(NB * SK, DM), 64),
        B_w_q.reshape(DM * NH, DH),
        B_w_uk.reshape(DM * NH, DH),
        B_w_uv.reshape(DM * NH, DH),
        _tile_major(B_w_o.reshape(NH * DH, DM), 16),
    )
    return out.reshape(NB, 1, 2 * DM)
```
